```python
import os as _os
_os.environ.setdefault("JAX_PLATFORMS", "cpu")
import jax
import jax.numpy as jnp

def _softmax(x, axis=-1):
    return jax.nn.softmax(x, axis=axis)
def _gelu(x):
    return jax.nn.gelu(x, approximate=True)
def _silu(x):
    return jax.nn.silu(x)
def _sigmoid(x):
    return jax.nn.sigmoid(x)
def _layernorm(x, axis=-1, eps=1e-5):
    m = jnp.mean(x, axis=axis, keepdims=True)
    v = jnp.var(x, axis=axis, keepdims=True)
    return (x - m) / jnp.sqrt(v + eps)
def _scatter_add(tgt, idx, src, axis=0):
    return tgt.at[idx].add(src)
def _segment_sum(src, seg, n):
    return jax.ops.segment_sum(src, seg, n)
class _Rng:
    def __init__(self, key):
        self._k = key
    def _next(self):
        self._k, sub = jax.random.split(self._k)
        return sub
    def normal(self, shape):
        return jax.random.normal(self._next(), shape, dtype=jnp.bfloat16)
    def randint(self, lo, hi, shape):
        return jax.random.randint(self._next(), shape, lo, hi, dtype=jnp.int32)
    def uniform(self, shape, lo=0.0, hi=1.0):
        return jax.random.uniform(self._next(), shape, jnp.bfloat16, lo, hi)
    def permutation(self, n):
        return jax.random.permutation(self._next(), n)


kernel_name = 'interleave_layers__ssm_conv_h3__dense_activation_silu__prompt'

def setup_inputs():
    _rng = _Rng(jax.random.key(int.from_bytes(__import__("os").urandom(4), "little")))
    _w = (lambda a: (lambda t: t.astype(jnp.bfloat16) if jnp.issubdtype(t.dtype, jnp.floating) else t)(jnp.asarray(a)))
    def _A_setup():
        B, S, D = 1, 2048, 448
        ks = 4
        return {
            "q": _w((lambda *s: _rng.normal(s) * 0.05)(B, S, D)),
            "k": _w((lambda *s: _rng.normal(s) * 0.2)(B, S, D)),
            "v": _w((lambda *s: _rng.normal(s) * 0.2)(B, S, D)),
            "shift_k": _w((lambda *s: _rng.normal(s) * 0.2)(D, ks) * 0.5),
            "ssm_k": _w((lambda *s: _rng.normal(s) * 0.2)(D, S) * (1.0 / S ** 0.5)),
            "ssm_D": _w((lambda *s: _rng.normal(s) * 0.2)(D)),
        }
    _A_in = _A_setup()

    def _B_setup():
        B, S, D, F = 1, 2048, 448, 1792
        return {
            "x": _w((lambda *s: _rng.normal(s) * 0.05)(B, S, D)),
            "w1": _w((lambda *s: _rng.normal(s) * 0.2)(D, F) * (D ** -0.5)),
            "w2": _w((lambda *s: _rng.normal(s) * 0.2)(F, D) * (F ** -0.5)),
        }
    _B_in = _B_setup()

    return {
        "A_q": _A_in["q"],
        "A_k": _A_in["k"],
        "A_v": _A_in["v"],
        "A_shift_k": _A_in["shift_k"],
        "A_ssm_k": _A_in["ssm_k"],
        "A_ssm_D": _A_in["ssm_D"],
        "B_x": _B_in["x"],
        "B_w1": _B_in["w1"],
        "B_w2": _B_in["w2"],
    }

def reference(A_q, A_k, A_v, A_shift_k, A_ssm_k, A_ssm_D, B_x, B_w1, B_w2):
    def _A_ref(q, k, v, shift_k, ssm_k, ssm_D):
        B, S, D = q.shape
        ks = shift_k.shape[-1]
        k_pad = jnp.pad(k, ((0, 0), (ks - 1, 0), (0, 0)))
        k_shift = jnp.zeros_like(k)
        for t in range(ks):
            k_shift = k_shift + k_pad[:, t:t + S, :] * shift_k[:, ks - 1 - t][None, None, :]
        kv = k_shift * v
        L = 2 * S
        kv_pad = jnp.pad(kv, ((0, 0), (0, S), (0, 0)))
        kf_pad = jnp.pad(ssm_k, ((0, 0), (0, S)))
        kv_f = (lambda x, axes=(-2,-1): jnp.fft.rfft2(x.astype(jnp.float32), axes=axes))(kv_pad[:, None, :, :], axes=(1, 2))
        kf_f = (lambda x, axes=(-2,-1): jnp.fft.rfft2(x.astype(jnp.float32), axes=axes))(kf_pad[:, None, :], axes=(1, 2))
        kf_f = (lambda x, *d: x.transpose(*d))(kf_f, 1, 2, 0)
        y_f = kv_f * kf_f[None, :, :, :]
        y = (lambda x, s, axes=(-2,-1): jnp.fft.irfft2(x, s=s, axes=axes).astype(jnp.bfloat16))(y_f, (1, L), axes=(1, 2))[:, 0, :S, :]
        y = y + kv * ssm_D[None, None, :]
        return q * y

    def _B_ref(x, w1, w2):
        h = jnp.einsum("bsd,df->bsf", x, w1)
        h = _silu(h)
        out = jnp.einsum("bsf,fd->bsd", h, w2)
        return out

    x = A_q
    x = x + _A_ref(_layernorm(x, axis=-1), A_k, A_v, A_shift_k, A_ssm_k, A_ssm_D)
    x = x + _B_ref(_layernorm(x, axis=-1), B_w1, B_w2)
    x = x + _A_ref(_layernorm(x, axis=-1), A_k, A_v, A_shift_k, A_ssm_k, A_ssm_D)
    x = x + _B_ref(_layernorm(x, axis=-1), B_w1, B_w2)
    return x
```

```python
import functools
import numpy as np
import jax
import jax.numpy as jnp
import jax.experimental.pallas as pl
import jax.experimental.pallas.tpu as pltpu

S, D, F = 2048, 448, 1792
B = 128
TM = 256
NB = S // B
NSTEP = S // TM
EPS = 1e-5
f32 = jnp.float32
bf16 = jnp.bfloat16
u32 = jnp.uint32
UB = 1
T1, T2, TC = 3584, 3136, 448
HB = NB + 3
GS = HB + NB + 2
NSLOT = GS + 1


def _tables():
    t = np.arange(B, dtype=np.float64)[:, None]
    g = np.arange(B, dtype=np.float64)[None, :]
    ang = 2.0 * np.pi * (g + 0.5) * t / (2 * B)
    fwd = np.concatenate([np.cos(ang), -np.sin(ang)], axis=1)
    inv = fwd.T / B
    return jnp.asarray(fwd, dtype=bf16), jnp.asarray(inv, dtype=bf16)


def _stats(x):
    m = jnp.sum(x, axis=0, keepdims=True) * (1.0 / D)
    xc = x - m
    v = jnp.sum(xc * xc, axis=0, keepdims=True) * (1.0 / D)
    return m, jax.lax.rsqrt(v + EPS)


def _ln(x):
    m, r = _stats(x)
    return (x - m) * r


def _silu(h):
    hh = 0.5 * h
    return hh + hh * jnp.tanh(hh)


def pk(x):
    return pltpu.bitcast(x, u32)


def upk(x):
    return pltpu.bitcast(x, bf16)


def make(LR=16, scopes=False, RA=160,
         winB=((100, 1500), (2100, 3000), (3700, 6600)), winK=((150, 6500),),
         g0=0, g1=216, lgate=None):

    def kernel(q_hbm, k_hbm, v_hbm, h_hbm, sk_hbm, dd_hbm, w1_hbm, w2_hbm, fwd_hbm, inv_hbm, o_hbm,
               q_buf, k_buf, v_buf, h_buf, sk_ref, dd_ref, w1_ref, w2_ref, fwd_ref, inv_ref, o_buf,
               sp_scr, kd_scr, uprev_scr, ktail_scr, taps_scr, w1t_scr, w2t_scr,
               hid0, hid1, hid2, hid3, x1_scr, y_scr, za_scr, flag_scr,
               sem_in, sem_misc, sem_out):
        hid_scr = (hid0, hid1, hid2, hid3)
        srcs = (q_hbm, k_hbm, v_hbm, h_hbm)
        bufs = (q_buf, k_buf, v_buf, h_buf)

        def blk_copy(which, c):
            return pltpu.make_async_copy(srcs[which].at[:, pl.ds(pl.multiple_of(c * TM, TM), TM)],
                                         bufs[which].at[c], sem_in.at[which, c])

        def out_copy(c):
            return pltpu.make_async_copy(o_buf.at[c], o_hbm.at[:, pl.ds(pl.multiple_of(c * TM, TM), TM)],
                                         sem_out.at[c])

        misc = [pltpu.make_async_copy(s, d, sem_misc.at[i]) for i, (s, d) in enumerate(
            [(fwd_hbm, fwd_ref), (sk_hbm, sk_ref), (dd_hbm, dd_ref), (inv_hbm, inv_ref),
             (w1_hbm, w1_ref), (w2_hbm, w2_ref)])]

        def conv_fwd_h(c, cs):
            n0 = 2 * c
            fwd = fwd_ref[...]
            for a in range(2):
                sp_scr[HB + n0 + a] = jnp.dot(h_buf[cs, :, a * B:(a + 1) * B], fwd, preferred_element_type=f32)

        def conv_kv(c, cs):
            out = []
            toks = []
            for r in range(0, D, LR):
                rows = pl.ds(r, LR)
                kf = k_buf[cs, rows, :].astype(f32)
                kext = jnp.concatenate([ktail_scr[rows, :], kf], axis=1)
                vf = v_buf[cs, rows, :].astype(f32)
                tap = [jnp.concatenate([taps_scr[j, rows, :]] * 2, axis=1) for j in range(5)]
                ks = kf * tap[0]
                for j in range(1, 4):
                    ks = ks + pltpu.roll(kext, j, axis=1)[:, B:] * tap[j]
                ktail_scr[rows, :] = kf[:, B:]
                kvf = ks * vf
                kv = [kvf[:, t * B:(t + 1) * B].astype(bf16) for t in range(2)]
                kd = jnp.concatenate([kv[0].astype(f32), kv[1].astype(f32)], axis=1) * tap[4]
                kd_scr[c % 2, rows, :] = kd
                out.append(kv)
                kb = pk(kd)
                toks.append((kb[:8, :B] | kb[8:, :B]) | (kb[:8, B:] | kb[8:, B:]))
            return [jnp.concatenate([o[t] for o in out], axis=0) for t in range(2)], toks

        def conv_fwd_u(c, kv):
            n0 = 2 * c
            fwd = fwd_ref[...]
            u0 = jnp.dot(kv[0], fwd, preferred_element_type=f32)
            u1 = jnp.dot(kv[1], fwd, preferred_element_type=f32)
            lane = jax.lax.broadcasted_iota(jnp.int32, (1, B), 1)
            sgn = (1 - 2 * (lane % 2)).astype(f32)
            up = uprev_scr[...]
            sp_scr[UB + n0, :, :B] = u0[:, :B] - sgn * up[:, B:]
            sp_scr[UB + n0, :, B:] = u0[:, B:] + sgn * up[:, :B]
            sp_scr[UB + n0 + 1, :, :B] = u1[:, :B] - sgn * u0[:, B:]
            sp_scr[UB + n0 + 1, :, B:] = u1[:, B:] + sgn * u0[:, :B]
            uprev_scr[...] = u1

        def conv_mac(c, nterms, r0, r1, release=None):
            n0 = 2 * c
            toks = []
            z = [[], []]
            for r in range(r0, r1, 8):
                rows = pl.ds(r, 8)
                for a in range(2):
                    for j in range(nterms):
                        if release is not None:
                            release(((r - r0) // 8 * 2 + a) * nterms + j)
                        hj = jnp.minimum(j, n0 + 1)
                        hr = sp_scr[HB + hj, rows, :B]
                        hi = sp_scr[HB + hj, rows, B:]
                        ui = jnp.maximum(n0 + a - j + UB, 0)
                        ur = sp_scr[ui, rows, :B]
                        uim = sp_scr[ui, rows, B:]
                        if j == 0:
                            ar, ai = ur * hr - uim * hi, ur * hi + uim * hr
                        else:
                            ar, ai = (ar + ur * hr) - uim * hi, (ai + ur * hi) + uim * hr
                    z[a].append(jnp.concatenate([ar, ai], axis=1))
                    toks.append(pk(ar) | pk(ai))
            return [jnp.concatenate(z[a], axis=0) for a in range(2)], toks

        def gated(w_scr, gates, never):
            ng = w_scr.shape[0] // 8
            byg = {}
            for (g, kt), tok in gates.items():
                byg.setdefault(g, {})[kt] = tok
            parts = []
            start = 0
            for g in sorted(byg) + [ng]:
                if g > start:
                    parts.append(w_scr[start * 8:g * 8, :])
                if g < ng:
                    p = w_scr[g * 8:(g + 1) * 8, :]
                    cols = []
                    c0 = 0
                    for kt in sorted(byg[g]):
                        if kt * 128 > c0:
                            cols.append(p[:, c0:kt * 128])
                        cols.append(jnp.where(never, byg[g][kt], p[:, kt * 128:(kt + 1) * 128]))
                        c0 = (kt + 1) * 128
                    if c0 < p.shape[1]:
                        cols.append(p[:, c0:])
                    parts.append(jnp.concatenate(cols, axis=1) if len(cols) > 1 else cols[0])
                start = g + 1
            return upk(jnp.concatenate(parts, axis=0) if len(parts) > 1 else parts[0])

        def conv_inv(c, z, cs):
            inv = inv_ref[...]
            yc = jnp.concatenate([jnp.dot(z[a].astype(bf16), inv, preferred_element_type=f32) for a in range(2)],
                                 axis=1)
            y = yc + kd_scr[c % 2]
            q = q_buf[cs].astype(f32)
            x1 = q + _ln(q) * y
            xn = _ln(x1)
            return y, x1, [xn[:, t * B:(t + 1) * B].astype(bf16) for t in range(2)]

        def mm1(xn, l, gates, never, zero):
            toks = []
            for t in range(2):
                h = _silu(jnp.dot(gated(w1t_scr, gates[t], never), xn[t], preferred_element_type=f32)).astype(bf16)
                hp = pk(h)
                hid_scr[2 * l + t][zero] = hp
                toks += [hp[g * 8:(g + 1) * 8] for g in range(F // 16)]
            return toks

        def mac_a(c, nterms, rtoks, zero):
            nt = (RA // 8) * 2 * nterms
            rtoks = rtoks[g0:g1]
            at = {}
            for i in range(len(rtoks)):
                at.setdefault(i * nt // len(rtoks), i)

            def release(idx):
                if idx in at:
                    sp_scr[GS + zero, 0:8, 0:B] = pltpu.bitcast(rtoks[at[idx]], f32)
            za, _ = conv_mac(c, nterms, 0, RA, release)
            for a in range(2):
                za_scr[a] = za[a]

        def mm2(l, gates, never, zero):
            return jnp.concatenate(
                [jnp.dot(gated(w2t_scr, gates[t], never), upk(hid_scr[2 * l + t][zero * 2]),
                         preferred_element_type=f32) for t in range(2)], axis=1)

        TL = [("2", 0, 2), ("3", T2, 1), ("4", T2 + T1 + 3 * TC, 2), ("1", 2 * T2 + T1 + 3 * TC, 1)]

        def place(toks, wins, gates):
            tot = sum(b - a for a, b in wins)
            n = len(toks)
            for i, tok in enumerate(toks):
                x = tot * (i + 1) / n
                for a, b in wins:
                    if x <= b - a:
                        t = int(a + x)
                        break
                    x -= b - a
                for name, st, kind in TL:
                    ln = T1 if kind == 1 else T2
                    if st <= t < st + ln:
                        t -= st
                        if kind == 1:
                            tt, key = t // 1792, ((t % 1792) // 16, 0)
                        else:
                            tile = (t // 448) * 4
                            tt, key = tile // 14, ((t % 448) // 16, tile % 14)
                        d = gates[name][tt]
                        d[key] = tok if key not in d else d[key] | tok
                        break
                else:
                    raise ValueError(t)

        def scoped(name, f):
            if scopes:
                with jax.named_scope(name):
                    return f()
            return f()

        def prologue():
            for cp in misc[:3]:
                cp.start()
            for w in (3, 1, 2, 0):
                blk_copy(w, 0).start()
            misc[3].start()
            misc[4].start()
            for w in (3, 1, 2):
                blk_copy(w, 1).start()
            misc[5].start()
            blk_copy(0, 1).start()
            for w in (1, 2, 3):
                blk_copy(w, 2).start()
            flag_scr[0] = 0
            zero = flag_scr[0]
            never = zero > 0
            ktail_scr[...] = jnp.zeros((D, B), f32)
            uprev_scr[...] = jnp.zeros((D, 2 * B), f32)
            sp_scr[0] = jnp.zeros((D, 2 * B), f32)
            for cp in misc[:3]:
                cp.wait()
            sk = sk_ref[...].astype(f32)
            dd = dd_ref[...].astype(f32).reshape(1, D)
            p = jnp.concatenate([sk, dd, jnp.zeros((3, D), f32)], axis=0)
            pt = p.T
            for j in range(5):
                taps_scr[j] = jnp.broadcast_to(pt[:, j:j + 1], (D, B))
            for w in (3, 1, 2, 0):
                blk_copy(w, 0).wait()
            misc[3].wait()
            conv_fwd_h(0, 0)
            conv_fwd_u(0, conv_kv(0, 0)[0])
            y, x1, xn = conv_inv(0, conv_mac(0, 2, 0, D)[0], 0)
            y_scr[...] = y
            x1_scr[...] = x1
            misc[4].wait()
            w1t_scr[...] = pk(w1_ref[...].T)
            for w in (3, 1, 2):
                blk_copy(w, 1).wait()
            conv_fwd_h(1, 1)
            conv_fwd_u(1, conv_kv(1, 1)[0])
            mac_a(1, 4, mm1(xn, 0, ({}, {}), never, zero), zero)
            misc[5].wait()
            w2t_scr[...] = pk(w2_ref[...])

        def body(m, with_conv):
            zero = flag_scr[0]
            never = zero > 0
            gates = {k: ({}, {}) for k in "1234"}
            x1 = x1_scr[...]
            y = y_scr[...]
            if with_conv:
                cs2 = jnp.minimum(m + 2, NSTEP - 1)
                zb, toks = conv_mac(m + 1, NB, RA, D)
                place(toks, winB, gates)
                z = [jnp.concatenate([za_scr[a], zb[a]], axis=0) for a in range(2)]
                kv, toks = conv_kv(m + 2, cs2)
                place(toks, winK, gates)
            x2 = x1 + mm2(0, gates["2"], never, zero)
            x3 = x2 + _ln(x2) * y
            xn3 = _ln(x3)
            mm1([xn3[:, t * B:(t + 1) * B].astype(bf16) for t in range(2)], 1, gates["3"], never, zero)
            if with_conv:
                yn, x1n, xn = conv_inv(m + 1, z, m + 1)
                y_scr[...] = yn
                x1_scr[...] = x1n
                conv_fwd_h(m + 2, cs2)
                conv_fwd_u(m + 2, kv)
                if lgate is not None:
                    tk = [pk(xn[t]) for t in range(2)]
                    lt = [tk[0][g * 8:(g + 1) * 8] | tk[1][g * 8:(g + 1) * 8] for g in range(D // 16)]
                    place(lt, (lgate,), gates)
            o_buf[m] = (x3 + mm2(1, gates["4"], never, zero)).astype(bf16)
            if with_conv:
                mac_a(m + 2, NB, mm1(xn, 0, gates["1"], never, zero), zero)

        scoped("prologue", prologue)

        def step(m, carry):
            blk_copy(0, m + 1).wait()

            @pl.when(m + 2 < NSTEP)
            def _():
                for w in (1, 2, 3):
                    blk_copy(w, m + 2).wait()
                blk_copy(0, m + 2).start()

            @pl.when(m + 3 < NSTEP)
            def _():
                for w in (1, 2, 3):
                    blk_copy(w, m + 3).start()

            scoped("main", lambda: body(m, True))
            out_copy(m).start()
            return carry

        jax.lax.fori_loop(0, NSTEP - 1, step, 0)
        scoped("last", lambda: body(NSTEP - 1, False))
        out_copy(NSTEP - 1).start()
        for c in range(NSTEP):
            out_copy(c).wait()

    @jax.jit
    def run(A_q, A_k, A_v, A_shift_k, A_ssm_k, A_ssm_D, B_x, B_w1, B_w2):
        qT = jnp.swapaxes(A_q, 1, 2).reshape(D, S)
        kT = jnp.swapaxes(A_k, 1, 2).reshape(D, S)
        vT = jnp.swapaxes(A_v, 1, 2).reshape(D, S)
        fwd, inv = _tables()
        anyspec = pl.BlockSpec(memory_space=pl.ANY)
        out = pl.pallas_call(
            kernel,
            in_specs=[anyspec] * 10,
            out_specs=anyspec,
            out_shape=jax.ShapeDtypeStruct((D, S), bf16),
            scratch_shapes=[
                pltpu.VMEM((NSTEP, D, TM), bf16), pltpu.VMEM((NSTEP, D, TM), bf16),
                pltpu.VMEM((NSTEP, D, TM), bf16), pltpu.VMEM((NSTEP, D, TM), bf16),
                pltpu.VMEM((4, D), bf16), pltpu.VMEM((D,), bf16),
                pltpu.VMEM((D, F), bf16), pltpu.VMEM((D, F), bf16),
                pltpu.VMEM((B, 2 * B), bf16), pltpu.VMEM((2 * B, B), bf16),
                pltpu.VMEM((NSTEP, D, TM), bf16),
                pltpu.VMEM((NSLOT, D, 2 * B), f32),
                pltpu.VMEM((2, D, TM), f32),
                pltpu.VMEM((D, 2 * B), f32),
                pltpu.VMEM((D, B), f32),
                pltpu.VMEM((5, D, B), f32),
                pltpu.VMEM((F // 2, D), u32),
                pltpu.VMEM((D // 2, F), u32),
                pltpu.VMEM((1, F // 2, B), u32), pltpu.VMEM((1, F // 2, B), u32),
                pltpu.VMEM((1, F // 2, B), u32), pltpu.VMEM((1, F // 2, B), u32),
                pltpu.VMEM((D, TM), f32),
                pltpu.VMEM((D, TM), f32),
                pltpu.VMEM((2, RA, 2 * B), f32),
                pltpu.SMEM((1,), jnp.int32),
                pltpu.SemaphoreType.DMA((4, NSTEP)),
                pltpu.SemaphoreType.DMA((6,)),
                pltpu.SemaphoreType.DMA((NSTEP,)),
            ],
            compiler_params=pltpu.CompilerParams(vmem_limit_bytes=100 * 1024 * 1024),
        )(qT, kT, vT, A_ssm_k, A_shift_k.T, A_ssm_D, B_w1, B_w2.T, fwd, inv)
        return jnp.swapaxes(out.reshape(1, D, S), 1, 2)
    return run


_impl = make()


@jax.jit
def pallas_interleave_layers__ssm_conv_h3__dense_activation_silu__prompt_kernel(
    A_q: jax.Array,
    A_k: jax.Array,
    A_v: jax.Array,
    A_shift_k: jax.Array,
    A_ssm_k: jax.Array,
    A_ssm_D: jax.Array,
    B_x: jax.Array,
    B_w1: jax.Array,
    B_w2: jax.Array,
):
    return _impl(A_q, A_k, A_v, A_shift_k, A_ssm_k, A_ssm_D, B_x, B_w1, B_w2)
```

```python
import functools
import numpy as np
import jax
import jax.numpy as jnp
import jax.experimental.pallas as pl
import jax.experimental.pallas.tpu as pltpu

S, D, F = 2048, 448, 1792
B = 128
TM = 256
NB = S // B
NSTEP = S // TM
EPS = 1e-5
f32 = jnp.float32
bf16 = jnp.bfloat16
u32 = jnp.uint32
T1, T2, TC = 3584, 3136, 448
UB = 1
HB = UB + NB
GS = HB + NB
NSLOT = GS + 1
CH2 = (((0, 4, 0), (4, 8, 1), (8, 12, 2), (12, 14, 3)), ((0, 2, 3), (2, 6, 4), (6, 10, 5), (10, 14, 6)))
NSEM = 8


def _tables():
    t = np.arange(B, dtype=np.float64)[:, None]
    g = np.arange(B, dtype=np.float64)[None, :]
    ang = 2.0 * np.pi * (g + 0.5) * t / (2 * B)
    fwd = np.concatenate([np.cos(ang), -np.sin(ang)], axis=1)
    inv = fwd.T / B
    return jnp.asarray(fwd, dtype=bf16), jnp.asarray(inv, dtype=bf16)


def _silu(h):
    hh = 0.5 * h
    return hh + hh * jnp.tanh(hh)


def pk(x):
    return pltpu.bitcast(x, u32)


def upk(x):
    return pltpu.bitcast(x, bf16)


def pack_pairs(x):
    n, c = x.shape[0] // 16, x.shape[1]
    x3 = x.reshape(n, 16, c)
    p = pltpu.pack_elementwise([x3[:, :8], x3[:, 8:]], packed_dtype=bf16)
    return p.reshape(n * 8, c)


def make(LR=16, scopes=False, WC=128, LG=32, LGP=448, OSPLIT=4,
         rel=((5400, 13300), (14100, 14600)), winK=(150, 3400), qgate=(2600, 3000)):

    def kernel(q_hbm, k_hbm, v_hbm, h_hbm, sk_hbm, dd_hbm, w1_hbm, w2_hbm, fwd_hbm, inv_hbm, o_hbm,
               q_buf, k_buf, v_buf, h_buf, sk_ref, dd_ref, w1_ref, w2_ref, fwd_ref, inv_ref, o_buf,
               sp_scr, kd_scr, uprev_scr, ktail_scr, taps_scr, w1t_scr, w2t_scr,
               hid0, hid1, hid2, hid3, la0, la1, lb0, lb1, st_scr, z_scr, flag_scr,
               sem_in, sem_out):
        hid_scr = (hid0, hid1, hid2, hid3)
        la, lb = (la0, la1), (lb0, lb1)
        srcs = (q_hbm, k_hbm, v_hbm, h_hbm)
        bufs = (q_buf, k_buf, v_buf, h_buf)

        def Z(i):
            return flag_scr[i]

        def blk_group(which, c):
            need = c - 1 if which == 0 else c - 2
            if c == 0:
                return 1 if which in (1, 2) else 2
            return 4 if need < 0 else (6 if need == 0 else 7)

        def blk_copy(which, c):
            return pltpu.make_async_copy(srcs[which].at[:, pl.ds(c * TM, TM)],
                                         bufs[which].at[c], sem_in.at[blk_group(which, c)])

        def out_copy(c, t, r0=0, r1=D):
            col = c * TM + t * B if isinstance(c, int) else pl.multiple_of(c * TM + t * B, B)
            return pltpu.make_async_copy(o_buf.at[2 * c + t, r0:r1], o_hbm.at[r0:r1, pl.ds(col, B)], sem_out.at[0])

        misc = [pltpu.make_async_copy(s, d, sem_in.at[g]) for (s, d, g) in
                [(fwd_hbm, fwd_ref, 2), (sk_hbm, sk_ref, 0), (dd_hbm, dd_ref, 0), (inv_hbm, inv_ref, 2),
                 (w1_hbm, w1_ref, 3), (w2_hbm, w2_ref, 5)]]

        def scoped(name, f):
            if scopes:
                with jax.named_scope(name):
                    return f()
            return f()

        def conv_fwd_h(c):
            fwd = fwd_ref[...]
            for a in range(2):
                sp_scr[HB + 2 * c + a] = jnp.dot(h_buf[c, :, a * B:(a + 1) * B], fwd, preferred_element_type=f32)

        def conv_kv(c):
            out = []
            toks = []
            for r in range(0, D, LR):
                rows = pl.ds(r, LR)
                kf = k_buf[c, rows, :].astype(f32)
                kext = jnp.concatenate([ktail_scr[rows, :], kf], axis=1)
                vf = v_buf[c, rows, :].astype(f32)
                tap = [jnp.concatenate([taps_scr[j, rows, :]] * 2, axis=1) for j in range(5)]
                ks = kf * tap[0]
                for j in range(1, 4):
                    ks = ks + pltpu.roll(kext, j, axis=1)[:, B:] * tap[j]
                ktail_scr[rows, :] = kf[:, B:]
                kvf = ks * vf
                kv = [kvf[:, t * B:(t + 1) * B].astype(bf16) for t in range(2)]
                kd = jnp.concatenate([kv[0].astype(f32), kv[1].astype(f32)], axis=1) * tap[4]
                kd_scr[c % 2, rows, :] = kd
                out.append(kv)
                kb = pk(kd)
                toks.append((kb[:8, :B] | kb[8:, :B]) | (kb[:8, B:] | kb[8:, B:]))
            return [jnp.concatenate([o[t] for o in out], axis=0) for t in range(2)], toks

        def conv_fwd_u(c, kv):
            n0 = 2 * c
            fwd = fwd_ref[...]
            u0 = jnp.dot(kv[0], fwd, preferred_element_type=f32)
            u1 = jnp.dot(kv[1], fwd, preferred_element_type=f32)
            lane = jax.lax.broadcasted_iota(jnp.int32, (1, B), 1)
            sgn = (1 - 2 * (lane % 2)).astype(f32)
            up = uprev_scr[...]
            sp_scr[UB + n0, :, :B] = u0[:, :B] - sgn * up[:, B:]
            sp_scr[UB + n0, :, B:] = u0[:, B:] + sgn * up[:, :B]
            sp_scr[UB + n0 + 1, :, :B] = u1[:, :B] - sgn * u0[:, B:]
            sp_scr[UB + n0 + 1, :, B:] = u1[:, B:] + sgn * u0[:, :B]
            uprev_scr[...] = u1

        class Mac:
            def __init__(self, c, nterms):
                self.c, self.nterms = c, nterms
                self.total = (D // 8) * nterms
                self.idx = 0
                self.acc = None
                self.prev_u = None

            def term(self):
                c, n0 = self.c, 2 * self.c
                r, j = (self.idx // self.nterms) * 8, self.idx % self.nterms
                self.idx += 1
                rows = pl.ds(r, 8)
                static = isinstance(c, int)
                hj = HB + (min(j, n0 + 1) + Z(0) if static else jnp.minimum(j, n0 + 1))
                hr = sp_scr[hj, rows, :B]
                hi = sp_scr[hj, rows, B:]
                if j == 0:
                    self.acc = {}
                for a in (1, 0):
                    if a == 1 and j > 0:
                        ur, uim = self.prev_u
                    else:
                        ui = max(n0 + a - j + UB, 0) + Z(0) if static else jnp.maximum(n0 + a - j + UB, 0)
                        ur = sp_scr[ui, rows, :B]
                        uim = sp_scr[ui, rows, B:]
                    if a == 0:
                        self.prev_u = (ur, uim)
                    if j == 0:
                        self.acc[a] = (ur * hr - uim * hi, ur * hi + uim * hr)
                    else:
                        ar, ai = self.acc[a]
                        self.acc[a] = ((ar + ur * hr) - uim * hi, (ai + ur * hi) + uim * hr)
                if j == self.nterms - 1:
                    for a in range(2):
                        z_scr[a + Z(3), rows, :B] = self.acc[a][0]
                        z_scr[a + Z(3), rows, B:] = self.acc[a][1]

            def run(self, toks, upto):
                end = int(round(self.total * upto))
                n = end - self.idx
                start = self.idx
                for i, tok in enumerate(toks):
                    tgt = start + (i + 1) * n // len(toks)
                    if self.idx < tgt:
                        sp_scr[GS + Z(1), 0:8, 0:B] = tok
                    while self.idx < tgt:
                        self.term()
                while self.idx < end:
                    self.term()

        def gated(w, gates, never):
            parts = []
            start = 0
            ng = w.shape[0] // 8
            for g in sorted(gates) + [ng]:
                if g > start:
                    parts.append(w[start * 8:g * 8, :])
                if g < ng:
                    p = w[g * 8:(g + 1) * 8, :]
                    parts.append(jnp.concatenate([jnp.where(never, gates[g], p[:, :128]), p[:, 128:]], axis=1))
                start = g + 1
            return jnp.concatenate(parts, axis=0) if len(parts) > 1 else parts[0]

        class Stats:
            def __init__(self, shift, s1=None, s2=None):
                self.c, self.s1, self.s2 = shift, s1, s2

            def add(self, x):
                for r in range(0, x.shape[0], 8):
                    d = x[r:r + 8] - self.c
                    self.s1 = d if self.s1 is None else self.s1 + d
                    self.s2 = d * d if self.s2 is None else self.s2 + d * d

            def done(self):
                m1 = jnp.sum(self.s1, axis=0, keepdims=True) * (1.0 / D)
                m2 = jnp.sum(self.s2, axis=0, keepdims=True) * (1.0 / D)
                var = jnp.maximum(m2 - m1 * m1, 0.0)
                return self.c + m1, jax.lax.rsqrt(var + EPS)

        def norm_pass(buf, src, dst, mean, rstd, lg):
            for i, r in enumerate(range(0, D, lg)):
                x = buf[src + Z(2 + i % 2), r:r + lg, :]
                n = ((x - mean) * rstd).astype(bf16)
                buf[dst + Z(4), r // 2:(r + lg) // 2, :] = pltpu.bitcast(pk(n), f32)

        def load_packed(buf, slot):
            return upk(pltpu.bitcast(buf[slot + Z(5), 0:D // 2, :], u32))

        def q_stats(c):
            res = []
            for t in range(2):
                cols = slice(t * B, (t + 1) * B)
                sq = Stats(q_buf[c, 0:16, cols].astype(f32)[0:1])
                for r in range(0, D, 16):
                    sq.add(q_buf[c, r:r + 16, cols].astype(f32))
                res.append(sq.done())
            return res

        def conv_inv(c, qs, lg):
            inv = inv_ref[...]
            means = []
            for t in range(2):
                cols = slice(t * B, (t + 1) * B)
                mq, rq = qs[t]
                yc = jnp.dot(z_scr[t + Z(3)].astype(bf16), inv, preferred_element_type=f32)
                s1 = Stats(mq)
                for r in range(0, D, 16):
                    y = yc[r:r + 16] + kd_scr[c % 2, r:r + 16, cols]
                    q = q_buf[c + Z(6), r:r + 16, cols].astype(f32)
                    x1 = q + ((q - mq) * rq) * y
                    la[t][0 + Z(4), r:r + 16, :] = y
                    la[t][1 + Z(4), r:r + 16, :] = x1
                    s1.add(x1)
                m1, r1 = s1.done()
                norm_pass(la[t], 1, 2, m1, r1, lg)
                means.append(m1)
            return means

        def mid_first(t, x2, mean1):
            st = Stats(mean1)
            for r in range(0, D, 16):
                lb[t][0 + Z(4), r:r + 16, :] = x2[r:r + 16]
                st.add(x2[r:r + 16])
            return st

        def mid_rest(t, st2):
            m2, r2 = st2.done()
            st = Stats(m2)
            for i, r in enumerate(range(0, D, LG)):
                x2 = lb[t][0 + Z(2 + i % 2), r:r + LG, :]
                y = la[t][0 + Z(7), r:r + LG, :]
                x3 = x2 + ((x2 - m2) * r2) * y
                lb[t][1 + Z(4), r:r + LG, :] = x3
                st.add(x3)
            m3, r3 = st.done()
            norm_pass(lb[t], 1, 2, m3, r3, LG)

        def mm1(xn, l, t, t_start=0, w=None, rows=(0, F)):
            w = w1t_scr[Z(7), rows[0] // 2:rows[1] // 2, :] if w is None else w
            h = _silu(jnp.dot(upk(w), xn, preferred_element_type=f32))
            hid_scr[2 * l + t][Z(0), rows[0] // 2:rows[1] // 2, :] = pack_pairs(h)
            return [(t_start + t * 1792 + rows[0] + g * 16, h[g * 16 + 8:g * 16 + 16])
                    for g in range((rows[1] - rows[0]) // 16)]

        def mm2(x, l, t, t_start=0, w=None):
            toks = []
            acc = x
            for (ka, kb, rnd) in CH2[t]:
                wc = w2t_scr[Z(7), :, ka * 128:kb * 128] if w is None else w[:, ka * 128:kb * 128]
                h = upk(hid_scr[2 * l + t][Z(6), ka * 64:kb * 64, :])
                acc = acc + jnp.dot(upk(wc), h, preferred_element_type=f32)
                if not (t == 1 and rnd == 3):
                    toks += [(t_start + rnd * 448 + g * 16, acc[g * 16 + 8:g * 16 + 16]) for g in range(D // 16)]
            return acc, toks

        def pick(toks, wins):
            return [tok for (t, tok) in toks if any(a <= t < b for a, b in wins)]

        def s2_tile(t, mean1, t_start, w=None):
            x2, toks = mm2(la[t][1 + Z(6)], 0, t, t_start, w=w)
            st = mid_first(t, x2, mean1)
            if t == 0:
                mid_rest(0, st)
            else:
                st_scr[0] = st.s1
                st_scr[1] = st.s2
                st_scr[2] = jnp.broadcast_to(st.c, (8, B))
            return toks

        def w1_prep(c0, c1):
            wparts = []
            for c in range(c0, c1, WC):
                wt = pk(w1_ref[:, c:c + WC].T).reshape(WC // 16, 8, D)
                lo = pltpu.unpack_elementwise(wt, index=0, packed_dtype=bf16, unpacked_dtype=f32)
                hi = pltpu.unpack_elementwise(wt, index=1, packed_dtype=bf16, unpacked_dtype=f32)
                wp = pk(jnp.concatenate([lo, hi], axis=1).reshape(WC, D).astype(bf16))
                w1t_scr[0, c // 2:(c + WC) // 2, :] = wp
                wparts.append(wp)
            return jnp.concatenate(wparts, axis=0)

        def prologue():
            for i in (1, 2):
                misc[i].start()
            blk_copy(1, 0).start()
            blk_copy(2, 0).start()
            misc[0].start()
            blk_copy(3, 0).start()
            blk_copy(0, 0).start()
            misc[3].start()
            misc[4].start()
            for w in (1, 2, 3):
                blk_copy(w, 1).start()
            misc[5].start()
            for c in range(1, NSTEP):
                blk_copy(0, c).start()
                if c + 1 < NSTEP:
                    for w in (1, 2, 3):
                        blk_copy(w, c + 1).start()
            for i in range(8):
                flag_scr[i] = 0
            ktail_scr[...] = jnp.zeros((D, B), f32)
            uprev_scr[...] = jnp.zeros((D, 2 * B), f32)
            sp_scr[0] = jnp.zeros((D, 2 * B), f32)
            scoped("w_small", lambda: [cp.wait() for cp in misc[1:3]])
            sk = sk_ref[...].astype(f32)
            dd = dd_ref[...].astype(f32).reshape(1, D)
            p = jnp.concatenate([sk, dd, jnp.zeros((3, D), f32)], axis=0)
            pt = p.T
            for j in range(5):
                taps_scr[j] = jnp.broadcast_to(pt[:, j:j + 1], (D, B))
            scoped("w_kv0", lambda: [blk_copy(w, 0).wait() for w in (1, 2)])
            kv = conv_kv(0)[0]
            scoped("w_blk0", lambda: [misc[0].wait()] + [blk_copy(w, 0).wait() for w in (3, 0)] + [misc[3].wait()])
            conv_fwd_u(0, kv)
            conv_fwd_h(0)
            Mac(0, 2).run([], 1.0)
            means = conv_inv(0, q_stats(0), LGP)
            scoped("w_w1", lambda: misc[4].wait())
            mm1(load_packed(la[0], 2), 0, 0, w=w1_prep(0, F))
            scoped("w_blk1", lambda: [blk_copy(w, 1).wait() for w in (1, 2, 3)])
            conv_fwd_h(1)
            conv_fwd_u(1, conv_kv(1)[0])
            toks = mm1(load_packed(la[1], 2), 0, 1)
            Mac(1, 4).run(pick(toks, ((1792, 3400),)), 1.0)
            scoped("w_w2", lambda: misc[5].wait())
            w2p = pk(w2_ref[...])
            w2t_scr[0] = w2p
            s2_tile(0, means[0], 0, w=w2p)
            s2_tile(1, means[1], 0)
            scoped("w_blk2", lambda: [blk_copy(0, 1).wait()] + [blk_copy(w, 2).wait() for w in (1, 2, 3)])

        def body(m, nxt, fwd):
            never = Z(0) > 0
            t4 = T1 + (TC if nxt else 0) + (2 * TC if fwd else 0)
            gates = ({}, {})

            def deadline(tok, t):
                d, g = gates[t // 1792], (t % 1792) // 16
                d[g] = tok if g not in d else d[g] | tok

            if fwd:
                kv, toks = conv_kv(m + 2)
                for i, tok in enumerate(toks):
                    deadline(tok, int(winK[0] + (winK[1] - winK[0]) * (i + 1) / len(toks)))
            if nxt:
                qs = q_stats(m + 1)
                for t in range(2):
                    deadline(pk(jnp.broadcast_to(qs[t][1], (8, B))), qgate[t])
            w1t = w1t_scr.at[Z(7)]
            mm1(load_packed(lb[0], 2), 1, 0, w=gated(w1t, gates[0], never))
            mid_rest(1, Stats(st_scr[2][0:1], st_scr[0], st_scr[1]))
            mm1(load_packed(lb[1], 2), 1, 1, w=gated(w1t, gates[1], never))
            if nxt:
                means = conv_inv(m + 1, qs, LG)
            if fwd:
                conv_fwd_h(m + 2)
                conv_fwd_u(m + 2, kv)
                mac = Mac(m + 2, NB)
            tot = sum(b - a for a, b in rel)

            def frac(t):
                return sum(max(0, min(b, t) - a) for a, b in rel) / tot

            toks = []
            for t in range(2):
                x4, tk = mm2(lb[t][1 + Z(6)], 1, t, t4)
                if nxt or t == 0:
                    o_buf[2 * m + t] = x4.astype(bf16)
                    out_copy(m, t).start()
                else:
                    for r in range(0, D, D // OSPLIT):
                        o_buf[2 * m + t, r:r + D // OSPLIT] = x4[r:r + D // OSPLIT].astype(bf16)
                        out_copy(m, t, r, r + D // OSPLIT).start()
                toks += tk
            if fwd:
                mac.run(pick(toks, rel), frac(t4 + T2))
            if nxt:
                toks = mm1(load_packed(la[0], 2), 0, 0, t4 + T2) + mm1(load_packed(la[1], 2), 0, 1, t4 + T2)
                if fwd:
                    mac.run(pick(toks, rel), frac(t4 + T2 + T1))
                toks = s2_tile(0, means[0], t4 + T2 + T1) + s2_tile(1, means[1], t4 + T2 + T1)
                if fwd:
                    mac.run(pick(toks, rel), 1.0)

        scoped("prologue", prologue)

        def step(i, carry):
            @pl.when(i == 1)
            def _():
                for w in range(4):
                    rest = bufs[w].at[(2 if w == 0 else 3):NSTEP]
                    pltpu.make_async_copy(rest, rest, sem_in.at[7]).wait()

            scoped("main", lambda: body(i, True, True))
            return carry

        jax.lax.fori_loop(0, NSTEP - 2, step, 0)

        def tail():
            body(NSTEP - 2, True, False)
            body(NSTEP - 1, False, False)
        scoped("last", tail)
        pltpu.make_async_copy(o_buf, o_buf, sem_out.at[0]).wait()

    @jax.jit
    def run(A_q, A_k, A_v, A_shift_k, A_ssm_k, A_ssm_D, B_x, B_w1, B_w2):
        qT = jnp.swapaxes(A_q, 1, 2).reshape(D, S)
        kT = jnp.swapaxes(A_k, 1, 2).reshape(D, S)
        vT = jnp.swapaxes(A_v, 1, 2).reshape(D, S)
        fwd, inv = _tables()
        anyspec = pl.BlockSpec(memory_space=pl.ANY)
        out = pl.pallas_call(
            kernel,
            in_specs=[anyspec] * 10,
            out_specs=anyspec,
            out_shape=jax.ShapeDtypeStruct((D, S), bf16),
            scratch_shapes=[
                pltpu.VMEM((NSTEP, D, TM), bf16), pltpu.VMEM((NSTEP, D, TM), bf16),
                pltpu.VMEM((NSTEP, D, TM), bf16), pltpu.VMEM((NSTEP, D, TM), bf16),
                pltpu.VMEM((4, D), bf16), pltpu.VMEM((D,), bf16),
                pltpu.VMEM((D, F), bf16), pltpu.VMEM((D, F), bf16),
                pltpu.VMEM((B, 2 * B), bf16), pltpu.VMEM((2 * B, B), bf16),
                pltpu.VMEM((2 * NSTEP, D, B), bf16),
                pltpu.VMEM((NSLOT, D, 2 * B), f32),
                pltpu.VMEM((2, D, TM), f32),
                pltpu.VMEM((D, 2 * B), f32),
                pltpu.VMEM((D, B), f32),
                pltpu.VMEM((5, D, B), f32),
                pltpu.VMEM((1, F // 2, D), u32),
                pltpu.VMEM((1, D // 2, F), u32),
                pltpu.VMEM((1, F // 2, B), u32), pltpu.VMEM((1, F // 2, B), u32),
                pltpu.VMEM((1, F // 2, B), u32), pltpu.VMEM((1, F // 2, B), u32),
                pltpu.VMEM((3, D, B), f32), pltpu.VMEM((3, D, B), f32),
                pltpu.VMEM((3, D, B), f32), pltpu.VMEM((3, D, B), f32),
                pltpu.VMEM((3, 8, B), f32),
                pltpu.VMEM((2, D, 2 * B), f32),
                pltpu.SMEM((8,), jnp.int32),
                pltpu.SemaphoreType.DMA((NSEM,)),
                pltpu.SemaphoreType.DMA((1,)),
            ],
            compiler_params=pltpu.CompilerParams(vmem_limit_bytes=100 * 1024 * 1024),
        )(qT, kT, vT, A_ssm_k, A_shift_k.T, A_ssm_D, B_w1, B_w2.T, fwd, inv)
        return jnp.swapaxes(out.reshape(1, D, S), 1, 2)
    return run


_impl = make()


@jax.jit
def pallas_interleave_layers__ssm_conv_h3__dense_activation_silu__prompt_kernel(
    A_q: jax.Array,
    A_k: jax.Array,
    A_v: jax.Array,
    A_shift_k: jax.Array,
    A_ssm_k: jax.Array,
    A_ssm_D: jax.Array,
    B_x: jax.Array,
    B_w1: jax.Array,
    B_w2: jax.Array,
):
    return _impl(A_q, A_k, A_v, A_shift_k, A_ssm_k, A_ssm_D, B_x, B_w1, B_w2)
```

```python
import numpy as np
import jax
import jax.numpy as jnp
import jax.experimental.pallas as pl
import jax.experimental.pallas.tpu as pltpu

S, D, F = 2048, 448, 1792
B = 128
TM = 2 * B
NB = S // B
NSTEP = S // TM
EPS = 1e-5
f32 = jnp.float32
bf16 = jnp.bfloat16
u32 = jnp.uint32

UB = 1
HB = UB + NB
GS = HB + NB
NSLOT = GS + 1
NFLAG = 8
W1A = 1152
LG = 32
OSPLIT = 7
T1, T2, TC = 3584, 3136, 448
CH2 = (((0, 4, 0), (4, 8, 1), (8, 12, 2), (12, 14, 3)), ((0, 2, 3), (2, 6, 4), (6, 10, 5), (10, 14, 6)))
REL = ((5000, 13300), (14100, 14600))
KV_WIN = (150, 2500)
Q_GATE = (2900, 3200)


def _dft_table():
    t = np.arange(B, dtype=np.float64)[:, None]
    g = np.arange(B, dtype=np.float64)[None, :]
    ang = 2.0 * np.pi * (g + 0.5) * t / (2 * B)
    return np.concatenate([np.cos(ang), -np.sin(ang)], axis=1).astype(bf16)


def _silu(h):
    hh = 0.5 * h
    return hh + hh * jnp.tanh(hh)


def _pk(x):
    return pltpu.bitcast(x, u32)


def _upk(x):
    return pltpu.bitcast(x, bf16)


def _dot(a, b):
    return jnp.dot(a, b, preferred_element_type=f32)


class _Stats:
    def __init__(self, shift, s1=None, s2=None):
        self.c, self.s1, self.s2 = shift, s1, s2

    def add(self, x):
        for r in range(0, x.shape[0], 8):
            d = x[r:r + 8] - self.c
            self.s1 = d if self.s1 is None else self.s1 + d
            self.s2 = d * d if self.s2 is None else self.s2 + d * d

    def done(self):
        m1 = jnp.sum(self.s1, axis=0, keepdims=True) * (1.0 / D)
        m2 = jnp.sum(self.s2, axis=0, keepdims=True) * (1.0 / D)
        var = jnp.maximum(m2 - m1 * m1, 0.0)
        return self.c + m1, jax.lax.rsqrt(var + EPS)


def _kernel(q_hbm, k_hbm, v_hbm, h_hbm, sk_hbm, dd_hbm, w1_hbm, w2_hbm, fwd_hbm, o_hbm,
            q_buf, k_buf, v_buf, h_buf, sk_ref, dd_ref, w1a_ref, w1b_ref, w2_ref, fwd_ref, inv_ref, o_buf,
            sp_scr, kd_scr, uprev_scr, taps_scr, w1t_scr, w2t_scr,
            hid0, hid1, hid2, hid3, la0, la1, lb0, lb1, st_scr, z_scr, flag_scr,
            sem_in, sem_out):
    hid_scr = (hid0, hid1, hid2, hid3)
    la, lb = (la0, la1), (lb0, lb1)
    srcs = (q_hbm, k_hbm, v_hbm, h_hbm)
    bufs = (q_buf, k_buf, v_buf, h_buf)
    Z = []

    def load_flags():
        Z[:] = [flag_scr[i] for i in range(NFLAG)]

    def blk_copy(which, c):
        need = c - 1 if which == 0 else c - 2
        if c == 0:
            grp = 1 if which in (1, 2) else 2
        else:
            grp = 4 if need < 0 else (6 if need == 0 else 7)
        return pltpu.make_async_copy(srcs[which].at[:, pl.ds(c * TM, TM)], bufs[which].at[c], sem_in.at[grp])

    def out_copy(c, t, r0, r1):
        col = c * TM + t * B if isinstance(c, int) else pl.multiple_of(c * TM + t * B, B)
        return pltpu.make_async_copy(o_buf.at[2 * c + t, r0:r1], o_hbm.at[r0:r1, pl.ds(col, B)], sem_out.at[0])

    def out_rows(last):
        step = D // OSPLIT if last else D
        return [(r, r + step) for r in range(0, D, step)]

    cp_fwd, cp_sk, cp_dd, cp_w1a, cp_w1b, cp_w2 = [
        pltpu.make_async_copy(s, d, sem_in.at[g]) for (s, d, g) in
        [(fwd_hbm, fwd_ref, 2), (sk_hbm, sk_ref, 0), (dd_hbm, dd_ref, 0),
         (w1_hbm.at[:, 0:W1A], w1a_ref, 3), (w1_hbm.at[:, W1A:F], w1b_ref, 4), (w2_hbm, w2_ref, 5)]]

    def wait_all(cps):
        for cp in cps:
            cp.wait()
        load_flags()

    def conv_kv(c):
        out = []
        toks = []
        par = c % 2
        for r in range(0, D, 16):
            rows = pl.ds(r, 16)
            kf = k_buf[c, rows, :].astype(f32)
            if isinstance(c, int) and c == 0:
                kprev = jnp.zeros((16, B), f32)
            else:
                kprev = k_buf[c - 1, rows, B:].astype(f32)
            kext = jnp.concatenate([kprev, kf], axis=1)
            vf = v_buf[c, rows, :].astype(f32)
            tap = [jnp.concatenate([taps_scr[j, rows, :]] * 2, axis=1) for j in range(5)]
            ks = kf * tap[0]
            for j in range(1, 4):
                ks = ks + pltpu.roll(kext, j, axis=1)[:, B:] * tap[j]
            kvf = ks * vf
            kv = [kvf[:, t * B:(t + 1) * B].astype(bf16) for t in range(2)]
            kd = jnp.concatenate([kv[0].astype(f32), kv[1].astype(f32)], axis=1) * tap[4]
            kd_scr[par, rows, :] = kd
            out.append(kv)
            kb = _pk(kd)
            kb = kb[:8] | kb[8:]
            toks.append(kb[:, :B] | kb[:, B:])
        return [jnp.concatenate([o[t] for o in out], axis=0) for t in range(2)], toks

    def alt_sign():
        lane = jax.lax.broadcasted_iota(jnp.int32, (1, B), 1)
        return (1 - 2 * (lane % 2)).astype(f32)

    def conv_fwd_h(c):
        fwd = fwd_ref[...]
        for a in range(2):
            sp_scr[HB + 2 * c + a] = _dot(h_buf[c, :, a * B:(a + 1) * B], fwd)

    def conv_fwd_u(c, kv):
        fwd = fwd_ref[...]
        u0, u1 = _dot(kv[0], fwd), _dot(kv[1], fwd)
        sgn = alt_sign()
        up = uprev_scr[...]
        n0 = UB + 2 * c
        sp_scr[n0, :, :B] = u0[:, :B] - sgn * up[:, B:]
        sp_scr[n0, :, B:] = u0[:, B:] + sgn * up[:, :B]
        sp_scr[n0 + 1, :, :B] = u1[:, :B] - sgn * u0[:, B:]
        sp_scr[n0 + 1, :, B:] = u1[:, B:] + sgn * u0[:, :B]
        uprev_scr[...] = u1

    class Mac:
        def __init__(self, c, nterms):
            n0 = 2 * c
            if isinstance(c, int):
                self.hj = [HB + min(j, n0 + 1) + Z[0] for j in range(nterms)]
                self.ui = [max(n0 + 1 - j + UB, 0) + Z[0] for j in range(nterms + 1)]
            else:
                self.hj = [HB + jnp.minimum(j, n0 + 1) for j in range(nterms)]
                self.ui = [jnp.maximum(n0 + 1 - j + UB, 0) for j in range(nterms + 1)]
            self.zi = [a + Z[3] for a in range(2)]
            self.gi = GS + Z[1]
            self.nterms = nterms
            self.total = (D // 8) * nterms
            self.idx = 0

        def load(self, slot, rows):
            return sp_scr[slot, rows, :B], sp_scr[slot, rows, B:]

        def term(self):
            r, j = (self.idx // self.nterms) * 8, self.idx % self.nterms
            self.idx += 1
            rows = pl.ds(r, 8)
            hr, hi = self.load(self.hj[j], rows)
            u = [self.load(self.ui[j + 1], rows), self.load(self.ui[0], rows) if j == 0 else self.prev]
            self.prev = u[0]
            if j == 0:
                self.acc = [(ur * hr - ui * hi, ur * hi + ui * hr) for (ur, ui) in u]
            else:
                self.acc = [((ar + ur * hr) - ui * hi, (ai + ur * hi) + ui * hr)
                            for (ar, ai), (ur, ui) in zip(self.acc, u)]
            if j == self.nterms - 1:
                for a in range(2):
                    z_scr[self.zi[a], rows, :B] = self.acc[a][0]
                    z_scr[self.zi[a], rows, B:] = self.acc[a][1]

        def run(self, toks, upto):
            end = int(round(self.total * upto))
            start, n = self.idx, end - self.idx
            for i, tok in enumerate(toks):
                tgt = start + (i + 1) * n // len(toks)
                if self.idx < tgt:
                    sp_scr[self.gi, 0:8, 0:B] = tok()
                while self.idx < tgt:
                    self.term()
            while self.idx < end:
                self.term()

    def norm_pass(buf, mean, rstd, lg):
        src, dst = [1 + Z[2], 1 + Z[3]], 2 + Z[4]
        for i, r in enumerate(range(0, D, lg)):
            n = ((buf[src[i % 2], r:r + lg, :] - mean) * rstd).astype(bf16)
            buf[dst, r // 2:(r + lg) // 2, :] = pltpu.bitcast(_pk(n), f32)

    def load_xn(buf):
        return _upk(pltpu.bitcast(buf[2 + Z[5], 0:D // 2, :], u32))

    def q_stats(c):
        res = []
        for t in range(2):
            sq = None
            for r in range(0, D, 16):
                q = q_buf[c, r:r + 16, t * B:(t + 1) * B].astype(f32)
                sq = _Stats(q[0:1]) if sq is None else sq
                sq.add(q)
            res.append(sq.done())
        return res

    def conv_inv(c, qs, lg, zs=None):
        inv = inv_ref[...]
        means = []
        par, cq, d0, d1 = c % 2, c + Z[6], Z[4], 1 + Z[4]
        for t in range(2):
            cols = slice(t * B, (t + 1) * B)
            mq, rq = qs[t]
            yc = _dot((z_scr[t + Z[3]] if zs is None else zs[t]).astype(bf16), inv)
            s1 = _Stats(mq)
            for r in range(0, D, 16):
                y = yc[r:r + 16] + kd_scr[par, r:r + 16, cols]
                q = q_buf[cq, r:r + 16, cols].astype(f32)
                x1 = q + ((q - mq) * rq) * y
                la[t][d0, r:r + 16, :] = y
                la[t][d1, r:r + 16, :] = x1
                s1.add(x1)
            m1, r1 = s1.done()
            norm_pass(la[t], m1, r1, lg)
            means.append(m1)
        return means

    def first_conv(kv):
        never = Z[0] > 0
        qs = q_stats(0)
        fwd = fwd_ref[...]
        hs = []
        for a in range(2):
            hb = h_buf[0, :, a * B:(a + 1) * B]
            tok = _upk(_pk(jnp.broadcast_to(qs[a][1], (8, B))))
            hh = _dot(jnp.concatenate([hb[:D - 16], jnp.where(never, tok, hb[D - 16:])], axis=0), fwd)
            sp_scr[HB + a] = hh
            hs.append((hh[:, :B], hh[:, B:]))
        u0, u1 = _dot(kv[0], fwd), _dot(kv[1], fwd)
        sgn = alt_sign()
        a0 = (u0[:, :B], u0[:, B:])
        a1 = (u1[:, :B] - sgn * u0[:, B:], u1[:, B:] + sgn * u0[:, :B])
        sp_scr[UB] = u0
        sp_scr[UB + 1, :, :B] = a1[0]
        sp_scr[UB + 1, :, B:] = a1[1]
        uprev_scr[...] = u1

        def cmul(x, y):
            return x[0] * y[0] - x[1] * y[1], x[0] * y[1] + x[1] * y[0]
        z0 = cmul(a0, hs[0])
        p, q = cmul(a1, hs[0]), cmul(a0, hs[1])
        z1 = (p[0] + q[0], p[1] + q[1])
        return conv_inv(0, qs, D, zs=[jnp.concatenate(z, axis=1) for z in (z0, z1)])

    def mid_rest(t, st2):
        m2, r2 = st2.done()
        st = _Stats(m2)
        d1 = 1 + Z[4]
        for i, r in enumerate(range(0, D, LG)):
            x2 = lb[t][Z[2 + i % 2], r:r + LG, :]
            x3 = x2 + ((x2 - m2) * r2) * la[t][Z[7], r:r + LG, :]
            lb[t][d1, r:r + LG, :] = x3
            st.add(x3)
        m3, r3 = st.done()
        norm_pass(lb[t], m3, r3, LG)

    def rows_tok(x, g):
        return lambda: x[g * 16 + 8:g * 16 + 16]

    def gated_w1(gates, never):
        w = w1t_scr.at[Z[7]]
        parts = []
        start = 0
        ng = F // 16
        for g in sorted(gates) + [ng]:
            if g > start:
                parts.append(w[start * 8:g * 8, :])
            if g < ng:
                p = w[g * 8:(g + 1) * 8, :]
                parts.append(jnp.concatenate([jnp.where(never, gates[g], p[:, :128]), p[:, 128:]], axis=1))
            start = g + 1
        return jnp.concatenate(parts, axis=0) if len(parts) > 1 else parts[0]

    def mm1(xn, l, t, t_start=0, w=None, r0=0, r1=F):
        w = w1t_scr[Z[7], r0 // 2:r1 // 2, :] if w is None else w
        h = _silu(_dot(_upk(w), xn))
        hid_scr[2 * l + t][Z[0], r0 // 2:r1 // 2, :] = _pk(h.astype(bf16))
        return [(t_start + t * (T1 // 2) + g * 16, rows_tok(h, g)) for g in range((r1 - r0) // 16)]

    def mm2(x, l, t, t_start=0, w=None):
        toks = []
        acc = x
        for (ka, kb, rnd) in CH2[t]:
            wc = w2t_scr[Z[7], :, ka * 128:kb * 128] if w is None else w[:, ka * 128:kb * 128]
            acc = acc + _dot(_upk(wc), _upk(hid_scr[2 * l + t][Z[6], ka * 64:kb * 64, :]))
            if not (t == 1 and rnd == 3):
                toks += [(t_start + rnd * D + g * 16, rows_tok(acc, g)) for g in range(D // 16)]
        return acc, toks

    def w1_transposed(src, c0):
        parts = []
        for c in range(0, src.shape[1], 128):
            wp = _pk(src[:, c:c + 128].T)
            w1t_scr[0, (c0 + c) // 2:(c0 + c + 128) // 2, :] = wp
            parts.append(wp)
        return jnp.concatenate(parts, axis=0)

    def pick(toks, wins):
        return [tok for (t, tok) in toks if any(a <= t < b for a, b in wins)]

    def ffn1_out(t, mean1, t_start, w=None):
        x2, toks = mm2(la[t][1 + Z[6]], 0, t, t_start, w=w)
        lb[t][Z[4]] = x2
        st = _Stats(mean1)
        st.add(x2)
        if t == 0:
            mid_rest(0, st)
        else:
            st_scr[0] = st.s1
            st_scr[1] = st.s2
            st_scr[2] = jnp.broadcast_to(st.c, (8, B))
        return toks

    order = [cp_sk, cp_dd, blk_copy(1, 0), blk_copy(2, 0), cp_fwd, blk_copy(3, 0), blk_copy(0, 0),
             cp_w1a, blk_copy(3, 1), blk_copy(1, 1), blk_copy(2, 1), cp_w1b, cp_w2]
    for c in range(1, NSTEP):
        order.append(blk_copy(0, c))
        if c + 1 < NSTEP:
            order += [blk_copy(w, c + 1) for w in (1, 2, 3)]
    for cp in order:
        cp.start()
    for i in range(NFLAG):
        flag_scr[i] = 0
    sp_scr[0] = jnp.zeros((D, 2 * B), f32)

    wait_all([cp_sk, cp_dd])
    sk = sk_ref[...].astype(f32)
    dd = dd_ref[...].astype(f32).reshape(1, D)
    pt = jnp.concatenate([sk, dd, jnp.zeros((3, D), f32)], axis=0).T
    for j in range(5):
        taps_scr[j] = jnp.broadcast_to(pt[:, j:j + 1], (D, B))

    wait_all([blk_copy(1, 0), blk_copy(2, 0)])
    kv0 = conv_kv(0)[0]

    wait_all([cp_fwd, blk_copy(3, 0), blk_copy(0, 0)])
    inv_ref[...] = (fwd_ref[...].astype(f32).T * (1.0 / B)).astype(bf16)
    means0 = first_conv(kv0)

    wait_all([cp_w1a])
    mm1(load_xn(la[0]), 0, 0, w=w1_transposed(w1a_ref, 0), r1=W1A)
    mm1(load_xn(la[1]), 0, 1, r1=W1A)

    wait_all([blk_copy(3, 1), blk_copy(1, 1), blk_copy(2, 1), cp_w1b])
    conv_fwd_h(1)
    mm1(load_xn(la[0]), 0, 0, w=w1_transposed(w1b_ref, W1A), r0=W1A)
    conv_fwd_u(1, conv_kv(1)[0])
    toks0 = mm1(load_xn(la[1]), 0, 1, r0=W1A)
    mac1 = Mac(1, 4)
    mac1.run([tok for (_, tok) in toks0[:-6]], 0.5)

    wait_all([cp_w2])
    w2p = _pk(w2_ref[...])
    w2t_scr[0] = w2p
    toks0 = ffn1_out(0, means0[0], 0, w=w2p) + ffn1_out(1, means0[1], 0)
    mac1.run(pick(toks0, ((0, 1500),)), 1.0)

    wait_all([blk_copy(0, 1)] + [blk_copy(w, 2) for w in (1, 2, 3)])

    def body(m, nxt, fwd):
        load_flags()
        never = Z[0] > 0
        t4 = T1 + (TC if nxt else 0) + (2 * TC if fwd else 0)
        gates = ({}, {})

        def deadline(tok, t):
            d, g = gates[t // (T1 // 2)], (t % (T1 // 2)) // 16
            d[g] = tok if g not in d else d[g] | tok

        def frac(t):
            return sum(max(0, min(b, t) - a) for a, b in REL) / sum(b - a for a, b in REL)

        if fwd:
            kv, toks = conv_kv(m + 2)
            for i, tok in enumerate(toks):
                deadline(tok, int(KV_WIN[0] + (KV_WIN[1] - KV_WIN[0]) * (i + 1) / len(toks)))
        if nxt:
            qs = q_stats(m + 1)
            for t in range(2):
                deadline(_pk(jnp.broadcast_to(qs[t][1], (8, B))), Q_GATE[t])
        mm1(load_xn(lb[0]), 1, 0, w=gated_w1(gates[0], never))
        mid_rest(1, _Stats(st_scr[2][0:1], st_scr[0], st_scr[1]))
        mm1(load_xn(lb[1]), 1, 1, w=gated_w1(gates[1], never))
        if nxt:
            means = conv_inv(m + 1, qs, LG)
        if fwd:
            conv_fwd_h(m + 2)
            conv_fwd_u(m + 2, kv)
            mac = Mac(m + 2, NB)
        toks = []
        for t in range(2):
            x4, tk = mm2(lb[t][1 + Z[6]], 1, t, t4)
            for r0, r1 in out_rows(not nxt and t == 1):
                o_buf[2 * m + t, r0:r1] = x4[r0:r1].astype(bf16)
                out_copy(m, t, r0, r1).start()
            toks += tk
        if fwd:
            mac.run(pick(toks, REL), frac(t4 + T2))
        if nxt:
            toks = mm1(load_xn(la[0]), 0, 0, t4 + T2) + mm1(load_xn(la[1]), 0, 1, t4 + T2)
            if fwd:
                mac.run(pick(toks, REL), frac(t4 + T2 + T1))
            toks = ffn1_out(0, means[0], t4 + T2 + T1) + ffn1_out(1, means[1], t4 + T2 + T1)
            if fwd:
                mac.run(pick(toks, REL), 1.0)

    def step(m, carry):
        @pl.when(m == 1)
        def _():
            for w in range(4):
                for c in range(2 if w == 0 else 3, NSTEP):
                    blk_copy(w, c).wait()

        body(m, True, True)
        return carry

    jax.lax.fori_loop(0, NSTEP - 2, step, 0)
    body(NSTEP - 2, True, False)
    body(NSTEP - 1, False, False)
    for c in range(NSTEP):
        for t in range(2):
            for r0, r1 in out_rows((c, t) == (NSTEP - 1, 1)):
                out_copy(c, t, r0, r1).wait()


def _call(qT, kT, vT, ssm_k, shift_t, ssm_d, w1, w2t, interpret=False):
    anyspec = pl.BlockSpec(memory_space=pl.ANY)
    blocks = pltpu.VMEM((NSTEP, D, TM), bf16)
    hidden = pltpu.VMEM((1, F // 2, B), u32)
    lnbuf = pltpu.VMEM((3, D, B), f32)
    return pl.pallas_call(
        _kernel,
        in_specs=[anyspec] * 9,
        out_specs=anyspec,
        out_shape=jax.ShapeDtypeStruct((D, S), bf16),
        scratch_shapes=[
            blocks, blocks, blocks, blocks,
            pltpu.VMEM((4, D), bf16), pltpu.VMEM((D,), bf16),
            pltpu.VMEM((D, W1A), bf16), pltpu.VMEM((D, F - W1A), bf16),
            pltpu.VMEM((D, F), bf16),
            pltpu.VMEM((B, 2 * B), bf16), pltpu.VMEM((2 * B, B), bf16),
            pltpu.VMEM((2 * NSTEP, D, B), bf16),
            pltpu.VMEM((NSLOT, D, 2 * B), f32),
            pltpu.VMEM((2, D, TM), f32),
            pltpu.VMEM((D, 2 * B), f32),
            pltpu.VMEM((5, D, B), f32),
            pltpu.VMEM((1, F // 2, D), u32),
            pltpu.VMEM((1, D // 2, F), u32),
            hidden, hidden, hidden, hidden,
            lnbuf, lnbuf, lnbuf, lnbuf,
            pltpu.VMEM((3, 8, B), f32),
            pltpu.VMEM((2, D, 2 * B), f32),
            pltpu.SMEM((NFLAG,), jnp.int32),
            pltpu.SemaphoreType.DMA((8,)),
            pltpu.SemaphoreType.DMA((1,)),
        ],
        compiler_params=pltpu.CompilerParams(vmem_limit_bytes=100 * 1024 * 1024),
        interpret=interpret,
    )(qT, kT, vT, ssm_k, shift_t, ssm_d, w1, w2t, _dft_table())


@jax.jit
def pallas_interleave_layers__ssm_conv_h3__dense_activation_silu__prompt_kernel(
    A_q: jax.Array,
    A_k: jax.Array,
    A_v: jax.Array,
    A_shift_k: jax.Array,
    A_ssm_k: jax.Array,
    A_ssm_D: jax.Array,
    B_x: jax.Array,
    B_w1: jax.Array,
    B_w2: jax.Array,
):
    del B_x
    qT = jnp.swapaxes(A_q, 1, 2).reshape(D, S)
    kT = jnp.swapaxes(A_k, 1, 2).reshape(D, S)
    vT = jnp.swapaxes(A_v, 1, 2).reshape(D, S)
    out = _call(qT, kT, vT, A_ssm_k, A_shift_k.T, A_ssm_D, B_w1, B_w2.T)
    return jnp.swapaxes(out.reshape(1, D, S), 1, 2)
```

```python
import numpy as np
import jax
import jax.numpy as jnp
import jax.experimental.pallas as pl
import jax.experimental.pallas.tpu as pltpu

S, D, F = 2048, 448, 1792
B = 128
TM = 2 * B
NB = S // B
NSTEP = S // TM
DH, FH = D // 2, F // 2
EPS = 1e-5
f32 = jnp.float32
bf16 = jnp.bfloat16
u32 = jnp.uint32

UB = 1
HB = UB + NB
GS = HB + NB
NSLOT = GS + 1
NFLAG = 8
OSPLIT = 2
T1, T2, TC = 3136, 2744, 448
ORDER2 = (0, 1, 4, 2, 5, 3, 6)


def _chunks2():
    out = []
    tile = 0
    for p in ORDER2:
        k = 0
        while k < 7:
            n = min(4 - tile % 4, 7 - k)
            out.append((p, k, k + n, tile // 4))
            k += n
            tile += n
    return out


def _dft_table():
    t = np.arange(B, dtype=np.float64)[:, None]
    g = np.arange(B, dtype=np.float64)[None, :]
    ang = 2.0 * np.pi * (g + 0.5) * t / (2 * B)
    return np.concatenate([np.cos(ang), -np.sin(ang)], axis=1).astype(bf16)


def _silu(h):
    hh = 0.5 * h
    return hh + hh * jnp.tanh(hh)


def _pk(x):
    return pltpu.bitcast(x, u32)


def _upk(x):
    return pltpu.bitcast(x, bf16)


def _dot(a, b):
    return jnp.dot(a, b, preferred_element_type=f32)


def _strassen_lhs(a11, a12, a21, a22):
    g11, g12, g21, g22 = [a.astype(f32) for a in (a11, a12, a21, a22)]
    c = lambda v: _pk(v.astype(bf16))
    return [c(g11 + g22), c(g21 + g22), _pk(a11), _pk(a22), c(g11 + g12), c(g21 - g11), c(g12 - g22)]


class _Stats:
    def __init__(self, shift, s1=None, s2=None):
        self.c, self.s1, self.s2 = shift, s1, s2

    def add(self, x):
        for r in range(0, x.shape[0], 8):
            d = x[r:r + 8] - self.c
            self.s1 = d if self.s1 is None else self.s1 + d
            self.s2 = d * d if self.s2 is None else self.s2 + d * d

    def done(self):
        m1 = jnp.sum(self.s1, axis=0, keepdims=True) * (1.0 / D)
        m2 = jnp.sum(self.s2, axis=0, keepdims=True) * (1.0 / D)
        var = jnp.maximum(m2 - m1 * m1, 0.0)
        return self.c + m1, jax.lax.rsqrt(var + EPS)


def make(scopes=False, interp=False, WA=512, LG=32, hb16=False, xb16=True,
         REL=((4700, 5200, 1.0), (5200, 7200, 2.0), (7200, 9000, 1.3), (9000, 10300, 0.6), (10300, 12400, 2.0), (12400, 12800, 1.0)),
         KV_WIN=(1500, 3500), Q_GATE=(300, 400),
         mfrac=0.4, dyn1=(False, False), popg=99, R1S=1, popg4=99,
         PX0=(2030, 2600), PN0=(140, 440), PX1=(460, 760), PN1=(900, 1450), PNA=(3900, 5100), LGT=64):

    def _kernel(q_hbm, k_hbm, v_hbm, h_hbm, sk_hbm, dd_hbm, w1_hbm, w2_hbm, fwd_hbm, o_hbm,
                q_buf, k_buf, v_buf, h_buf, sk_ref, dd_ref, w1a_ref, w1b_ref, w2_ref, fwd_ref, inv_ref, o_buf,
                sp_scr, kd_scr, uprev_scr, taps_scr, a1_scr, a2_scr,
                he0, hl0, he1, hl1, xa0, xa1, xb0, xb1, na, nb_, la0, la1, lb0, lb1, st_scr, z_scr, flag_scr,
                sem_in, sem_out):
        hid = ((he0, hl0), (he1, hl1))
        la, lb = (la0, la1), (lb0, lb1)
        xo = {id(la): ((xa0, xa1), na), id(lb): ((xb0, xb1), nb_)}
        srcs = (q_hbm, k_hbm, v_hbm, h_hbm)
        bufs = (q_buf, k_buf, v_buf, h_buf)
        Z = []

        def load_flags():
            Z[:] = [flag_scr[i] for i in range(NFLAG)]

        def scoped(name, f):
            if scopes:
                with jax.named_scope(name):
                    return f()
            return f()

        def blk_copy(which, c):
            need = c - 1 if which == 0 else c - 2
            if c == 0:
                grp = 1 if which in (1, 2) else 2
            else:
                grp = 4 if need < 0 else (6 if need == 0 else 7)
            return pltpu.make_async_copy(srcs[which].at[:, pl.ds(c * TM, TM)], bufs[which].at[c], sem_in.at[grp])

        def out_copy(c, t, r0, r1):
            col = c * TM + t * B if isinstance(c, int) else pl.multiple_of(c * TM + t * B, B)
            return pltpu.make_async_copy(o_buf.at[2 * c + t, r0:r1], o_hbm.at[r0:r1, pl.ds(col, B)], sem_out.at[0])

        def out_rows(last):
            step = D // OSPLIT if last else D
            return [(r, r + step) for r in range(0, D, step)]

        cp_fwd, cp_sk, cp_dd, cp_w2 = [
            pltpu.make_async_copy(s, d, sem_in.at[g]) for (s, d, g) in
            [(fwd_hbm, fwd_ref, 2), (sk_hbm, sk_ref, 0), (dd_hbm, dd_ref, 0), (w2_hbm, w2_ref, 5)]]
        cp_w1a = [pltpu.make_async_copy(w1_hbm.at[:, i * FH:i * FH + WA], w1a_ref.at[i], sem_in.at[3])
                  for i in (1, 0)]
        cp_w1b = [pltpu.make_async_copy(w1_hbm.at[:, i * FH + WA:(i + 1) * FH], w1b_ref.at[i], sem_in.at[4])
                  for i in (1, 0)]

        def wait_all(name, cps):
            scoped(name, lambda: [cp.wait() for cp in cps])
            load_flags()

        def conv_kv(c):
            out = []
            toks = []
            par = c % 2
            for r in range(0, D, 16):
                rows = pl.ds(r, 16)
                kf = k_buf[c, rows, :].astype(f32)
                if isinstance(c, int) and c == 0:
                    kprev = jnp.zeros((16, B), f32)
                else:
                    kprev = k_buf[c - 1, rows, B:].astype(f32)
                kext = jnp.concatenate([kprev, kf], axis=1)
                vf = v_buf[c, rows, :].astype(f32)
                tap = [jnp.concatenate([taps_scr[j, rows, :]] * 2, axis=1) for j in range(5)]
                ks = kf * tap[0]
                for j in range(1, 4):
                    ks = ks + pltpu.roll(kext, j, axis=1)[:, B:] * tap[j]
                kvf = ks * vf
                kv = [kvf[:, t * B:(t + 1) * B].astype(bf16) for t in range(2)]
                kd = jnp.concatenate([kv[0].astype(f32), kv[1].astype(f32)], axis=1) * tap[4]
                kd_scr[par, rows, :] = kd
                out.append(kv)
                kb = _pk(kd)
                kb = kb[:8] | kb[8:]
                toks.append(kb[:, :B] | kb[:, B:])
            return [jnp.concatenate([o[t] for o in out], axis=0) for t in range(2)], toks

        def alt_sign():
            lane = jax.lax.broadcasted_iota(jnp.int32, (1, B), 1)
            return (1 - 2 * (lane % 2)).astype(f32)

        def conv_fwd_h(c, gates=None, never=None):
            fwd = fwd_ref[...]
            for a in range(2):
                hb = h_buf[c, :, a * B:(a + 1) * B]
                if gates is not None:
                    g, tok = gates[a]
                    hb = jnp.concatenate([hb[:g * 16], jnp.where(never, _upk(tok), hb[g * 16:g * 16 + 16]),
                                          hb[g * 16 + 16:]], axis=0)
                hh = _dot(hb, fwd)
                sp_scr[HB + 2 * c + a] = hh
            return [(g * 16, (lambda g: lambda: hh[g * 16 + 8:g * 16 + 16, :B])(g)) for g in range(D // 16)]

        def conv_fwd_u(c, kv, t0=0):
            fwd = fwd_ref[...]
            u0, u1 = _dot(kv[0], fwd), _dot(kv[1], fwd)
            sgn = alt_sign()
            up = uprev_scr[...]
            n0 = UB + 2 * c
            sp_scr[n0, :, :B] = u0[:, :B] - sgn * up[:, B:]
            sp_scr[n0, :, B:] = u0[:, B:] + sgn * up[:, :B]
            sp_scr[n0 + 1, :, :B] = u1[:, :B] - sgn * u0[:, B:]
            sp_scr[n0 + 1, :, B:] = u1[:, B:] + sgn * u0[:, :B]
            uprev_scr[...] = u1
            return [(t0 + g * 16, (lambda g: lambda: u1[g * 16 + 8:g * 16 + 16, :B])(g)) for g in range(D // 16)]

        class Mac:
            def __init__(self, c, nterms):
                n0 = 2 * c
                if isinstance(c, int):
                    self.hj = [HB + min(j, n0 + 1) + Z[0] for j in range(nterms)]
                    self.ui = [max(n0 + 1 - j + UB, 0) + Z[0] for j in range(nterms + 1)]
                else:
                    self.hj = [HB + jnp.minimum(j, n0 + 1) for j in range(nterms)]
                    self.ui = [jnp.maximum(n0 + 1 - j + UB, 0) for j in range(nterms + 1)]
                self.zi = [a + Z[3] for a in range(2)]
                self.gi = GS + Z[1]
                self.nterms = nterms
                self.total = (D // 8) * nterms
                self.idx = 0

            def load(self, slot, rows):
                return sp_scr[slot, rows, :B], sp_scr[slot, rows, B:]

            def term(self):
                r, j = (self.idx // self.nterms) * 8, self.idx % self.nterms
                self.idx += 1
                rows = pl.ds(r, 8)
                hr, hi = self.load(self.hj[j], rows)
                u = [self.load(self.ui[j + 1], rows), self.load(self.ui[0], rows) if j == 0 else self.prev]
                self.prev = u[0]
                if j == 0:
                    self.acc = [(ur * hr - ui * hi, ur * hi + ui * hr) for (ur, ui) in u]
                else:
                    self.acc = [((ar + ur * hr) - ui * hi, (ai + ur * hi) + ui * hr)
                                for (ar, ai), (ur, ui) in zip(self.acc, u)]
                if j == self.nterms - 1:
                    for a in range(2):
                        z_scr[self.zi[a], rows, :B] = self.acc[a][0]
                        z_scr[self.zi[a], rows, B:] = self.acc[a][1]

            def run(self, toks, frac):
                for t, tok in sorted(toks, key=lambda x: x[0]):
                    tgt = int(round(self.total * frac(t)))
                    if self.idx < tgt:
                        sp_scr[self.gi, 0:8, 0:B] = tok()
                    while self.idx < tgt:
                        self.term()

            def finish(self):
                while self.idx < self.total:
                    self.term()

        XOP = {1: (0, 0), 3: (0, 1), 2: (1, 0), 4: (1, 1), 0: (1, 2), 6: (1, 3), 5: (1, 4)}

        def pacer(buf, toks, win, n):
            sel = [tok for (t, tok) in sorted(toks or [], key=lambda x: x[0]) if win[0] <= t < win[1]] if toks else []

            def pace(i):
                if sel:
                    buf[3 + Z[1], 0:8, :] = sel[min(i * len(sel) // n, len(sel) - 1)]()
            return pace

        def norm_pass(bufs2, t, mean, rstd, lg, toks=None, win=None):
            buf = bufs2[t]
            obuf, nbuf = xo[id(bufs2)]
            pace = pacer(buf, toks, win, D // lg)
            src = [1 + Z[2], 1 + Z[3]]
            hg = lg // 2
            for i, r in enumerate(range(0, DH, hg)):
                pace(i)
                lo = (buf[src[i % 2], r:r + hg, :] - mean) * rstd
                hi = (buf[src[i % 2], DH + r:DH + r + hg, :] - mean) * rstd
                if t == 0:
                    nbuf[Z[4], r:r + hg, :] = lo
                    nbuf[Z[4], DH + r:DH + r + hg, :] = hi
                    ops = [lo, hi - lo]
                else:
                    b11 = nbuf[Z[6], r:r + hg, :]
                    b21 = nbuf[Z[6], DH + r:DH + r + hg, :]
                    ops = [lo - hi, hi, b11 + hi, b21 + hi, b11 + lo]
                for k, o in enumerate(ops):
                    if xb16:
                        obuf[t][k + Z[4], r:r + hg, :] = o.astype(bf16)
                    else:
                        obuf[t][k + Z[4], r // 2:(r + hg) // 2, :] = _pk(o.astype(bf16))

        def load_xop(bufs2, p):
            t, k = XOP[p]
            x = xo[id(bufs2)][0][t][k + Z[5]]
            return x if xb16 else _upk(x)

        def q_stats(c):
            res = []
            for t in range(2):
                sq = None
                for r in range(0, D, 16):
                    q = q_buf[c, r:r + 16, t * B:(t + 1) * B].astype(f32)
                    sq = _Stats(q[0:1]) if sq is None else sq
                    sq.add(q)
                res.append(sq.done())
            return res

        def conv_inv(c, qs, lg, zs=None, t0=0, defer=False):
            inv = inv_ref[...]
            means = []
            toks = []
            par, cq, d0, d1 = c % 2, c + Z[6], Z[4], 1 + Z[4]
            for t in range(2):
                cols = slice(t * B, (t + 1) * B)
                mq, rq = qs[t]
                yc = _dot((z_scr[t + Z[3]] if zs is None else zs[t]).astype(bf16), inv)
                s1 = _Stats(mq)
                for r in range(0, D, 16):
                    y = yc[r:r + 16] + kd_scr[par, r:r + 16, cols]
                    q = q_buf[cq, r:r + 16, cols].astype(f32)
                    x1 = q + ((q - mq) * rq) * y
                    la[t][d0, r:r + 16, :] = y
                    la[t][d1, r:r + 16, :] = x1
                    s1.add(x1)
                m1, r1 = s1.done()
                if defer:
                    means.append((m1, r1))
                    if t == 0:
                        toks += [(t0 + g * 16, rows_tok(yc, g)) for g in range(D // 16)]
                else:
                    norm_pass(la, t, m1, r1, lg)
                    means.append(m1)
            return (means, toks) if defer else means

        def first_conv(kv):
            never = Z[0] > 0
            qs = q_stats(0)
            fwd = fwd_ref[...]
            hs = []
            for a in range(2):
                hb = h_buf[0, :, a * B:(a + 1) * B]
                tok = _upk(_pk(jnp.broadcast_to(qs[a][1], (8, B))))
                hh = _dot(jnp.concatenate([hb[:D - 16], jnp.where(never, tok, hb[D - 16:])], axis=0), fwd)
                sp_scr[HB + a] = hh
                hs.append((hh[:, :B], hh[:, B:]))
            u0, u1 = _dot(kv[0], fwd), _dot(kv[1], fwd)
            sgn = alt_sign()
            a0 = (u0[:, :B], u0[:, B:])
            a1 = (u1[:, :B] - sgn * u0[:, B:], u1[:, B:] + sgn * u0[:, :B])
            sp_scr[UB] = u0
            sp_scr[UB + 1, :, :B] = a1[0]
            sp_scr[UB + 1, :, B:] = a1[1]
            uprev_scr[...] = u1

            def cmul(x, y):
                return x[0] * y[0] - x[1] * y[1], x[0] * y[1] + x[1] * y[0]
            z0 = cmul(a0, hs[0])
            p, q = cmul(a1, hs[0]), cmul(a0, hs[1])
            z1 = (p[0] + q[0], p[1] + q[1])
            return conv_inv(0, qs, D, zs=[jnp.concatenate(z, axis=1) for z in (z0, z1)])

        def mid_x3(t, st2, toks=None, win=None, LG=LG):
            pace = pacer(lb[t], toks, win, D // LG)
            ysrc, yslot = (la[0], Z[7]) if t == 0 else (lb[1], 2 + Z[7])
            m2, r2 = st2.done()
            st = _Stats(m2)
            d1 = 1 + Z[4]
            for i, r in enumerate(range(0, D, LG)):
                pace(i)
                x2 = lb[t][Z[2 + i % 2], r:r + LG, :]
                x3 = x2 + ((x2 - m2) * r2) * ysrc[yslot, r:r + LG, :]
                lb[t][d1, r:r + LG, :] = x3
                st.add(x3)
            return st

        def keep_y():
            lb[1][2 + Z[4]] = la[1][Z[5]]

        def save_stats(t, st):
            st_scr[3 * t] = st.s1
            st_scr[3 * t + 1] = st.s2
            st_scr[3 * t + 2] = jnp.broadcast_to(st.c, (8, B))

        def load_stats(t):
            return _Stats(st_scr[3 * t + 2][0:1], st_scr[3 * t], st_scr[3 * t + 1])

        def rows_tok(x, g):
            return lambda: x[g * 16 + 8:g * 16 + 16]

        def a1_rows(p, r0, r1, gates=None, never=None, dyn=True):
            w = a1_scr.at[p + Z[7] if dyn else p]
            parts = []
            start = r0 // 16
            ng = r1 // 16
            for g in sorted(gates or {}) + [ng]:
                if g > start:
                    parts.append(w[start * 8:g * 8, :])
                if g < ng:
                    x = w[g * 8:(g + 1) * 8, :]
                    parts.append(jnp.concatenate([jnp.where(never, gates[g], x[:, :128]), x[:, 128:]], axis=1))
                start = g + 1
            return jnp.concatenate(parts, axis=0) if len(parts) > 1 else parts[0]

        HOP = {0: (0, 2), 1: (0, 1), 4: (0, 0), 2: (1, 0), 5: (1, 1), 3: (1, 2), 6: (1, 3)}

        def put_hop(l, p, r0, r1, v):
            cls, k = HOP[p]
            if hb16:
                hid[l][cls][k + Z[0], r0:r1, :] = v.astype(bf16)
            else:
                hid[l][cls][k + Z[0], r0 // 2:r1 // 2, :] = _pk(v.astype(bf16))

        def get_hop(l, p, r0, r1):
            cls, k = HOP[p]
            if hb16:
                return hid[l][cls][k + Z[6], r0:r1, :]
            return _upk(hid[l][cls][k + Z[6], r0 // 2:r1 // 2, :])

        def mm1(xb, l, t0=0, lhs=None, r0=0, r1=FH, gates=None, never=None, hooks=None, split0=1):
            n = r1 - r0
            gates = gates or {}
            hooks = hooks or {}

            def prod(p, rnd, a=r0, b=r1):
                gt = {g: tk for g, tk in gates.get(rnd, {}).items() if a // 16 <= g < b // 16} if p in (1, 2, 0) else {}
                w = a1_rows(p, a, b, gt, never, dyn1[l]) if lhs is None else lhs[p][(a - r0) // 2:(b - r0) // 2]
                return _dot(_upk(w), load_xop(xb, p))

            def toks(x, rnd, scale=1):
                return [(t0 + rnd * n + g * 16 // scale, rows_tok(x, g)) for g in range(n // 16)]
            def keep(i, v):
                return lambda: v

            if split0 > 1:
                m2s, m4s = [], []
                pr = n // split0
                for i in range(split0):
                    a = r0 + i * pr
                    if i > 0:
                        for g, gp in ((0, pr // 16 - 9), (4, pr // 16 - 5), (8, pr // 16 - 1)):
                            tk = _pk(rows_tok(m2s[-1], gp)()) | _pk(rows_tok(m4s[-1], gp)())
                            d = gates.setdefault(0, {})
                            k = a // 16 + g
                            d[k] = tk if k not in d else d[k] | tk
                    m2s.append(prod(1, 0, a, a + pr))
                    m4s.append(prod(3, 0, a, a + pr))
                m2, m4 = jnp.concatenate(m2s, axis=0), jnp.concatenate(m4s, axis=0)
            else:
                m2, m4 = prod(1, 0), prod(3, 0)
            h21 = _silu(m2 + m4)
            put_hop(l, 4, r0, r1, h21)
            out = toks(h21, 0)
            m2, m4, h21 = keep(0, m2), keep(1, m4), keep(2, h21)
            hooks.get(0, lambda tk: None)(out)
            m3, m5 = prod(2, 1), prod(4, 1)
            h12 = _silu(m3 + m5)
            put_hop(l, 1, r0, r1, h12)
            put_hop(l, 0, r0, r1, h12 + h21())
            p11, p22 = m4() - m5, m3 - m2()
            out += toks(h12, 1)
            p11, p22, h12 = keep(3, p11), keep(4, p22), keep(5, h12)
            hooks.get(1, lambda tk: None)(out)
            m1, m7 = prod(0, 2), prod(6, 2)
            h11 = _silu((p11() + m1) + m7)
            p22 = p22() + m1
            put_hop(l, 2, r0, r1, h11 - h21())
            put_hop(l, 5, r0, r1, h12() + h11)
            out += toks(h11, 2)
            p22 = keep(6, p22)()
            mid = r0 + n // 2
            h22a = _silu(p22[:n // 2] + prod(5, 3, r0, mid))
            h22b = _silu(p22[n // 2:] + prod(5, 3, mid, r1))
            h22 = jnp.concatenate([h22a, h22b], axis=0)
            put_hop(l, 3, r0, r1, h22 - h12())
            put_hop(l, 6, r0, r1, h22 + h21())
            out += [(t0 + 3 * n + g * 16, rows_tok(h22a, g)) for g in range(n // 32)]
            return out

        def mm2(l, t0, res, tile_done, lhs=None, pop_from=99):
            toks = []
            M = {}
            ch = _chunks2()
            never = Z[0] > 0
            prev_round, cur_round = [], []
            for i, (p, ka, kb, rnd) in enumerate(ch):
                first_in_round = i == 0 or ch[i - 1][3] != rnd
                if first_in_round:
                    prev_round, cur_round = cur_round, []
                w = a2_scr[p + Z[7], :, ka * 128:kb * 128] if lhs is None else lhs[p][:, ka * 128:kb * 128]
                if first_in_round and rnd >= pop_from:
                    parts = []
                    start = 0
                    for g, gp in ((0, 5), (4, 9), (8, 13)):
                        tk = None
                        for x in prev_round:
                            y = _pk(rows_tok(x, gp)())
                            tk = y if tk is None else tk | y
                        if g > start:
                            parts.append(w[start * 8:g * 8])
                        x = w[g * 8:(g + 1) * 8]
                        x0 = jnp.where(never, tk, x[:, :128])
                        parts.append(jnp.concatenate([x0, x[:, 128:]], axis=1) if x.shape[1] > 128 else x0)
                        start = g + 1
                    parts.append(w[start * 8:])
                    w = jnp.concatenate(parts, axis=0)
                w = _upk(w)
                hb = get_hop(l, p, ka * 128, kb * 128)
                if i == len(ch) - 1:
                    r = jnp.concatenate([_dot(w[a:b], hb) for a, b in ((0, 64), (64, 128), (128, 176), (176, DH))],
                                        axis=0)
                else:
                    r = _dot(w, hb)
                if p not in M:
                    if p == 5:
                        r = (((res(0, 1) + M[0]) - M[1]) + M[2]) + r
                    elif p == 6:
                        r = (((res(1, 0) + M[0]) - M[4]) + M[3]) + r
                    M[p] = r
                else:
                    M[p] = M[p] + r
                cur_round.append(M[p])
                if first_in_round:
                    toks += [(t0 + rnd * DH + g * 16, rows_tok(M[p], g)) for g in range(DH // 16)]
                if p == 5 and kb == 7:
                    tile_done(0, (res(0, 0) + M[4]) + M[2], M[5], (0, 1))
            tile_done(1, M[6], (res(1, 1) + M[1]) + M[3], (1, 0))
            return toks

        def ffn1_out(means, t0, lhs=None, fast=False):
            def fin(t, lo, hi, order):
                st = _Stats(means[t])
                for h in order:
                    x2 = (lo, hi)[h]
                    lb[t][Z[4], h * DH:(h + 1) * DH, :] = x2
                    st.add(x2)
                sts[t] = st
            sts = {}
            toks = mm2(0, t0, lambda t, h: la[t][1 + Z[6], h * DH:(h + 1) * DH, :], fin, lhs, popg)
            if fast:
                st3 = mid_x3(0, sts[0], toks, (t0 + PX0[0], t0 + PX0[0] + 200), LGT)
                norm_pass(lb, 0, *st3.done(), LGT, toks, (t0 + PX0[0] + 250, t0 + PX0[0] + 450))
            else:
                save_stats(0, mid_x3(0, sts[0], toks, (t0 + PX0[0], t0 + PX0[1])))
            save_stats(1, sts[1])
            return toks

        def ffn2_out(m, t0, last):
            def fin(t, lo, hi, order):
                for h in order:
                    o_buf[2 * m + t, h * DH:(h + 1) * DH] = (lo, hi)[h].astype(bf16)
                    if last and t == 1:
                        out_copy(m, t, h * DH, (h + 1) * DH).start()
                if not (last and t == 1):
                    out_copy(m, t, 0, D).start()
            return mm2(1, t0, lambda t, h: lb[t][1 + Z[6], h * DH:(h + 1) * DH, :], fin, None, popg4)

        def w1_operands(src, c0):
            parts = [[] for _ in range(7)]
            for c in range(0, src.shape[2], 128):
                blk = [src[i, k * DH:(k + 1) * DH, c:c + 128].T for i in range(2) for k in range(2)]
                for p, wp in enumerate(_strassen_lhs(*blk)):
                    a1_scr[p, (c0 + c) // 2:(c0 + c + 128) // 2, :] = wp
                    parts[p].append(wp)
            return [jnp.concatenate(x, axis=0) for x in parts]

        def prologue():
            order = [cp_sk, cp_dd, blk_copy(1, 0), blk_copy(2, 0), cp_fwd, blk_copy(3, 0), blk_copy(0, 0)] \
                + cp_w1a + [blk_copy(3, 1), blk_copy(1, 1), blk_copy(2, 1)] + cp_w1b + [cp_w2]
            for c in range(1, NSTEP):
                order.append(blk_copy(0, c))
                if c + 1 < NSTEP:
                    order += [blk_copy(w, c + 1) for w in (1, 2, 3)]
            for cp in order:
                cp.start()
            for i in range(NFLAG):
                flag_scr[i] = 0
            sp_scr[0] = jnp.zeros((D, 2 * B), f32)

            wait_all("w_small", [cp_sk, cp_dd])
            sk = sk_ref[...].astype(f32)
            dd = dd_ref[...].astype(f32).reshape(1, D)
            pt = jnp.concatenate([sk, dd, jnp.zeros((3, D), f32)], axis=0).T
            for j in range(5):
                taps_scr[j] = jnp.broadcast_to(pt[:, j:j + 1], (D, B))

            wait_all("w_kv0", [blk_copy(1, 0), blk_copy(2, 0)])
            kv0 = conv_kv(0)[0]

            wait_all("w_blk0", [cp_fwd, blk_copy(3, 0), blk_copy(0, 0)])
            inv_ref[...] = (fwd_ref[...].astype(f32).T * (1.0 / B)).astype(bf16)
            means0 = first_conv(kv0)
            keep_y()

            wait_all("w_w1a", cp_w1a)
            mm1(la, 0, lhs=w1_operands(w1a_ref, 0), r1=WA)

            wait_all("w_w1b", [blk_copy(3, 1), blk_copy(1, 1), blk_copy(2, 1)] + cp_w1b)
            conv_fwd_h(1)
            kv1 = conv_kv(1)[0]
            toks0 = mm1(la, 0, lhs=w1_operands(w1b_ref, WA), r0=WA, hooks={1: lambda tk: conv_fwd_u(1, kv1)})
            nb = FH - WA
            mac1 = Mac(1, 4)
            mac1.run([x for x in toks0 if x[0] >= 2 * nb], lambda t: mfrac * (t - 2 * nb) / (1.5 * nb))

            wait_all("w_w2", [cp_w2])
            lhs2 = _strassen_lhs(w2_ref[:DH, :FH], w2_ref[:DH, FH:], w2_ref[DH:, :FH], w2_ref[DH:, FH:])
            for p in range(7):
                a2_scr[p] = lhs2[p]
            toks0 = ffn1_out(means0, 0, lhs2)
            mac1.run(toks0, lambda t: min(1.0, mfrac + (1 - mfrac) * t / 1800))
            mac1.finish()

            wait_all("w_blk2", [blk_copy(0, 1)] + [blk_copy(w, 2) for w in (1, 2, 3)])

        def body(m, nxt, fwd):
            load_flags()
            never = Z[0] > 0
            t3 = (TC if nxt else 0) + (TC if fwd else 0)
            t4 = t3 + T1 + (TC if fwd else 0)
            gates = {0: {}, 1: {}, 2: {}}

            def deadline(tok, t):
                d, g = gates[(t - t3) // FH], ((t - t3) % FH) // 16
                d[g] = tok if g not in d else d[g] | tok

            def frac(t):
                return sum(w * max(0, min(b, t) - a) for a, b, w in REL) / sum(w * (b - a) for a, b, w in REL)

            if nxt:
                qs = q_stats(m + 1)
            th, ti = [], []
            if fwd:
                th = conv_fwd_h(m + 2, [(Q_GATE[t] // 16, _pk(jnp.broadcast_to(qs[t][1], (8, B)))) for t in range(2)],
                                never)
            if nxt:
                norm_pass(lb, 0, *load_stats(0).done(), LG if fwd else LGT, th, PN0)
            if nxt:
                mr, ti = conv_inv(m + 1, qs, LG, t0=t3 - TC, defer=True)
                means = [x[0] for x in mr]
            st3 = mid_x3(1, load_stats(1), ti if fwd else None, PX1, LG if fwd else LGT)
            if fwd:
                kv, toks = conv_kv(m + 2)
                for i, tok in enumerate(toks):
                    deadline(tok, int(KV_WIN[0] + (KV_WIN[1] - KV_WIN[0]) * (i + 1) / len(toks)))
            sh = t3 - 2 * TC
            toks = mm1(lb, 1, t3, gates=gates, never=never, split0=R1S,
                       hooks={0: lambda tk: norm_pass(lb, 1, *st3.done(), LG if fwd else LGT, tk,
                                                     (PN1[0] + sh, PN1[1] + sh) if nxt else (200, 450))})
            if nxt:
                keep_y()
            if fwd:
                toks += conv_fwd_u(m + 2, kv, t3 + T1)
                mac = Mac(m + 2, NB)
            toks4 = ffn2_out(m, t4, not nxt)
            if nxt:
                half = (PNA[0] + PNA[1]) // 2
                sh2 = 0 if fwd else -2 * TC
                norm_pass(la, 0, *mr[0], LG, toks + toks4, (PNA[0] + sh2, half + sh2))
                norm_pass(la, 1, *mr[1], LG, toks + toks4, (half + sh2, PNA[1] + sh2))
            toks = toks4
            if fwd:
                mac.run(toks, frac)
            if nxt:
                toks = mm1(la, 0, t4 + T2)
                if fwd:
                    mac.run(toks, frac)
                toks = ffn1_out(means, t4 + T2 + T1, fast=not fwd)
                if fwd:
                    mac.run(toks, frac)
                    mac.finish()

        scoped("prologue", prologue)

        def step(m, carry):
            @pl.when(m == 1)
            def _():
                for w in range(4):
                    for c in range(2 if w == 0 else 3, NSTEP):
                        blk_copy(w, c).wait()

            scoped("main", lambda: body(m, True, True))
            return carry

        jax.lax.fori_loop(0, NSTEP - 2, step, 0)

        def tail():
            body(NSTEP - 2, True, False)
            body(NSTEP - 1, False, False)
        scoped("last", tail)
        for c in range(NSTEP):
            for t in range(2):
                for r0, r1 in out_rows((c, t) == (NSTEP - 1, 1)):
                    out_copy(c, t, r0, r1).wait()

    @jax.jit
    def run(A_q, A_k, A_v, A_shift_k, A_ssm_k, A_ssm_D, B_x, B_w1, B_w2):
        qT = jnp.swapaxes(A_q, 1, 2).reshape(D, S)
        kT = jnp.swapaxes(A_k, 1, 2).reshape(D, S)
        vT = jnp.swapaxes(A_v, 1, 2).reshape(D, S)
        anyspec = pl.BlockSpec(memory_space=pl.ANY)
        blocks = pltpu.VMEM((NSTEP, D, TM), bf16)
        hbuf = (lambda n: pltpu.VMEM((n, FH, B), bf16)) if hb16 else (lambda n: pltpu.VMEM((n, FH // 2, B), u32))
        lnbuf = pltpu.VMEM((4, D, B), f32)
        xbuf = (lambda n: pltpu.VMEM((n, DH, B), bf16)) if xb16 else (lambda n: pltpu.VMEM((n, DH // 2, B), u32))
        out = pl.pallas_call(
            _kernel,
            in_specs=[anyspec] * 9,
            out_specs=anyspec,
            out_shape=jax.ShapeDtypeStruct((D, S), bf16),
            scratch_shapes=[
                blocks, blocks, blocks, blocks,
                pltpu.VMEM((4, D), bf16), pltpu.VMEM((D,), bf16),
                pltpu.VMEM((2, D, WA), bf16), pltpu.VMEM((2, D, FH - WA), bf16),
                pltpu.VMEM((D, F), bf16),
                pltpu.VMEM((B, 2 * B), bf16), pltpu.VMEM((2 * B, B), bf16),
                pltpu.VMEM((2 * NSTEP, D, B), bf16),
                pltpu.VMEM((NSLOT, D, 2 * B), f32),
                pltpu.VMEM((2, D, TM), f32),
                pltpu.VMEM((D, 2 * B), f32),
                pltpu.VMEM((5, D, B), f32),
                pltpu.VMEM((7, FH // 2, DH), u32),
                pltpu.VMEM((7, DH // 2, FH), u32),
                hbuf(3), hbuf(4), hbuf(3), hbuf(4),
                xbuf(2), xbuf(5), xbuf(2), xbuf(5), pltpu.VMEM((1, D, B), f32), pltpu.VMEM((1, D, B), f32),
                lnbuf, lnbuf, lnbuf, lnbuf,
                pltpu.VMEM((6, 8, B), f32),
                pltpu.VMEM((2, D, 2 * B), f32),
                pltpu.SMEM((NFLAG,), jnp.int32),
                pltpu.SemaphoreType.DMA((8,)),
                pltpu.SemaphoreType.DMA((1,)),
            ],
            compiler_params=pltpu.CompilerParams(vmem_limit_bytes=100 * 1024 * 1024),
            interpret=interp,
        )(qT, kT, vT, A_ssm_k, A_shift_k.T, A_ssm_D, B_w1, B_w2.T, _dft_table())
        return jnp.swapaxes(out.reshape(1, D, S), 1, 2)
    return run


_impl = make()


@jax.jit
def pallas_interleave_layers__ssm_conv_h3__dense_activation_silu__prompt_kernel(
    A_q: jax.Array,
    A_k: jax.Array,
    A_v: jax.Array,
    A_shift_k: jax.Array,
    A_ssm_k: jax.Array,
    A_ssm_D: jax.Array,
    B_x: jax.Array,
    B_w1: jax.Array,
    B_w2: jax.Array,
):
    return _impl(A_q, A_k, A_v, A_shift_k, A_ssm_k, A_ssm_D, B_x, B_w1, B_w2)
```

```python
import numpy as np
import jax
import jax.numpy as jnp
import jax.experimental.pallas as pl
import jax.experimental.pallas.tpu as pltpu

S, D, F = 2048, 448, 1792
B = 128
TM = 2 * B
NB = S // B
NSTEP = S // TM
DH, FH = D // 2, F // 2
EPS = 1e-5
f32 = jnp.float32
bf16 = jnp.bfloat16
u32 = jnp.uint32

UB = 1
HB = UB + NB
GS = HB + NB
NSLOT = GS + 1
NFLAG = 8
OSPLIT = 2
T1, T2, TC = 3136, 2744, 448
ORDER2 = (0, 1, 4, 2, 5, 3, 6)


def _chunks2():
    out = []
    tile = 0
    for p in ORDER2:
        k = 0
        while k < 7:
            n = min(4 - tile % 4, 7 - k)
            out.append((p, k, k + n, tile // 4))
            k += n
            tile += n
    return out


def _dft_table():
    t = np.arange(B, dtype=np.float64)[:, None]
    g = np.arange(B, dtype=np.float64)[None, :]
    ang = 2.0 * np.pi * (g + 0.5) * t / (2 * B)
    return np.concatenate([np.cos(ang), -np.sin(ang)], axis=1).astype(bf16)


def _silu(h):
    hh = 0.5 * h
    return hh + hh * jnp.tanh(hh)


def _pk(x):
    return pltpu.bitcast(x, u32)


def _upk(x):
    return pltpu.bitcast(x, bf16)


def _dot(a, b):
    return jnp.dot(a, b, preferred_element_type=f32)


def _strassen_lhs(a11, a12, a21, a22):
    g11, g12, g21, g22 = [a.astype(f32) for a in (a11, a12, a21, a22)]
    c = lambda v: _pk(v.astype(bf16))
    return [c(g11 + g22), c(g21 + g22), _pk(a11), _pk(a22), c(g11 + g12), c(g21 - g11), c(g12 - g22)]


class _Stats:
    def __init__(self, shift, s1=None, s2=None):
        self.c, self.s1, self.s2 = shift, s1, s2

    def add(self, x, cuts=None):
        cuts = cuts or (0, x.shape[0])
        for a, b in zip(cuts[:-1], cuts[1:]):
            p1 = p2 = None
            if len(cuts) == 2:
                p1, p2 = self.s1, self.s2
            for r in range(a, b, 8):
                d = x[r:r + 8] - self.c
                p1 = d if p1 is None else p1 + d
                p2 = d * d if p2 is None else p2 + d * d
            if len(cuts) == 2:
                self.s1, self.s2 = p1, p2
            else:
                self.s1, self.s2 = self.s1 + p1, self.s2 + p2

    def done(self):
        m1 = jnp.sum(self.s1, axis=0, keepdims=True) * (1.0 / D)
        m2 = jnp.sum(self.s2, axis=0, keepdims=True) * (1.0 / D)
        var = jnp.maximum(m2 - m1 * m1, 0.0)
        return self.c + m1, jax.lax.rsqrt(var + EPS)


def make(scopes=False, interp=False, WA=512, LG=32, hb16=False, xb16=True,
         REL=((4600, 5200, 1.2), (5200, 7000, 1.9), (7300, 9000, 1.5), (9000, 10200, 0.8), (10400, 12300, 1.9), (12300, 12600, 1.0)),
         KV_WIN=(1500, 3500), Q_GATE=(300, 400),
         mfrac=0.4, dyn1=(False, False), popg=99, R1S=1, popg4=99,
         PX0=(2030, 2600), PN0=(140, 440), PX1=(60, 400), PN1=(800, 1400), PNA=(3900, 5100), LGT=64, dyn2=(True, True), zdyn=False, hdyn=False, xdyn=True, NCH=4, d2tail=False, G=64, stage=True, FX=(2030, 2200, 2260, 2430), TX=(0, 250, 400, 900, 330, 600), TQ=(500, 600)):

    def _kernel(q_hbm, k_hbm, v_hbm, h_hbm, sk_hbm, dd_hbm, w1_hbm, w2_hbm, fwd_hbm, o_hbm,
                q_buf, k_buf, v_buf, h_buf, sk_ref, dd_ref, w1a_ref, w1b_ref, w2_ref, fwd_ref, inv_ref, o_buf,
                sp_scr, kd_scr, uprev_scr, taps_scr, a1_scr, a2_scr,
                he0, hl0, he1, hl1, pp, xa0, xa1, xb0, xb1, na, nb_, la0, la1, lb0, lb1, lx0, lx1, st_scr, z_scr, flag_scr,
                sem_in, sem_out):
        hid = ((he0, hl0), (he1, hl1))
        la, lb = (la0, la1), (lb0, lb1)
        lx = (lx0, lx1)
        xo = {id(la): ((xa0, xa1), na), id(lb): ((xb0, xb1), nb_)}
        srcs = (q_hbm, k_hbm, v_hbm, h_hbm)
        bufs = (q_buf, k_buf, v_buf, h_buf)
        Z = []
        MODE = {'mac': True}

        def load_flags():
            Z[:] = [flag_scr[i] for i in range(NFLAG)]

        def scoped(name, f):
            if scopes:
                with jax.named_scope(name):
                    return f()
            return f()

        def blk_copy(which, c):
            need = c - 1 if which == 0 else c - 2
            if c == 0:
                grp = 1 if which in (1, 2) else 2
            else:
                grp = 4 if need < 0 else (6 if need == 0 else 7)
            return pltpu.make_async_copy(srcs[which].at[:, pl.ds(c * TM, TM)], bufs[which].at[c], sem_in.at[grp])

        def out_copy(c, t, r0, r1):
            col = c * TM + t * B if isinstance(c, int) else pl.multiple_of(c * TM + t * B, B)
            return pltpu.make_async_copy(o_buf.at[2 * c + t, r0:r1], o_hbm.at[r0:r1, pl.ds(col, B)], sem_out.at[0])

        def out_rows(last):
            step = D // OSPLIT if last else D
            return [(r, r + step) for r in range(0, D, step)]

        cp_fwd, cp_sk, cp_dd, cp_w2 = [
            pltpu.make_async_copy(s, d, sem_in.at[g]) for (s, d, g) in
            [(fwd_hbm, fwd_ref, 2), (sk_hbm, sk_ref, 0), (dd_hbm, dd_ref, 0), (w2_hbm, w2_ref, 5)]]
        cp_w1a = [pltpu.make_async_copy(w1_hbm.at[:, i * FH:i * FH + WA], w1a_ref.at[i], sem_in.at[3])
                  for i in (1, 0)]
        cp_w1b = [pltpu.make_async_copy(w1_hbm.at[:, i * FH + WA:(i + 1) * FH], w1b_ref.at[i], sem_in.at[4])
                  for i in (1, 0)]

        def wait_all(name, cps):
            scoped(name, lambda: [cp.wait() for cp in cps])
            load_flags()

        def conv_kv(c):
            out = []
            toks = []
            par = c % 2
            for r in range(0, D, 16):
                rows = pl.ds(r, 16)
                kf = k_buf[c, rows, :].astype(f32)
                if isinstance(c, int) and c == 0:
                    kprev = jnp.zeros((16, B), f32)
                else:
                    kprev = k_buf[c - 1, rows, B:].astype(f32)
                kext = jnp.concatenate([kprev, kf], axis=1)
                vf = v_buf[c, rows, :].astype(f32)
                tap = [jnp.concatenate([taps_scr[j, rows, :]] * 2, axis=1) for j in range(5)]
                ks = kf * tap[0]
                for j in range(1, 4):
                    ks = ks + pltpu.roll(kext, j, axis=1)[:, B:] * tap[j]
                kvf = ks * vf
                kv = [kvf[:, t * B:(t + 1) * B].astype(bf16) for t in range(2)]
                kd = jnp.concatenate([kv[0].astype(f32), kv[1].astype(f32)], axis=1) * tap[4]
                kd_scr[par, rows, :] = kd
                out.append(kv)
                kb = _pk(kd)
                kb = kb[:8] | kb[8:]
                toks.append(kb[:, :B] | kb[:, B:])
            return [jnp.concatenate([o[t] for o in out], axis=0) for t in range(2)], toks

        def alt_sign():
            lane = jax.lax.broadcasted_iota(jnp.int32, (1, B), 1)
            return (1 - 2 * (lane % 2)).astype(f32)

        def conv_fwd_h(c, gates=None, never=None):
            fwd = fwd_ref[...]
            for a in range(2):
                hb = h_buf[c, :, a * B:(a + 1) * B]
                if gates is not None:
                    g, tok = gates[a]
                    hb = jnp.concatenate([hb[:g * 16], jnp.where(never, _upk(tok), hb[g * 16:g * 16 + 16]),
                                          hb[g * 16 + 16:]], axis=0)
                hh = _dot(hb, fwd)
                sp_scr[HB + 2 * c + a] = hh
            return [(g * 16, (lambda g: lambda: hh[g * 16 + 8:g * 16 + 16, :B])(g)) for g in range(D // 16)]

        def conv_fwd_u(c, kv, t0=0):
            fwd = fwd_ref[...]
            u0, u1 = _dot(kv[0], fwd), _dot(kv[1], fwd)
            sgn = alt_sign()
            up = uprev_scr[...]
            n0 = UB + 2 * c
            sp_scr[n0, :, :B] = u0[:, :B] - sgn * up[:, B:]
            sp_scr[n0, :, B:] = u0[:, B:] + sgn * up[:, :B]
            sp_scr[n0 + 1, :, :B] = u1[:, :B] - sgn * u0[:, B:]
            sp_scr[n0 + 1, :, B:] = u1[:, B:] + sgn * u0[:, :B]
            uprev_scr[...] = u1
            return [(t0 + g * 16, (lambda g: lambda: u1[g * 16 + 8:g * 16 + 16, :B])(g)) for g in range(D // 16)]

        class Mac:
            def __init__(self, c, nterms):
                n0 = 2 * c
                if isinstance(c, int):
                    self.hj = [HB + min(j, n0 + 1) + Z[0] for j in range(nterms)]
                    self.ui = [max(n0 + 1 - j + UB, 0) + Z[0] for j in range(nterms + 1)]
                else:
                    self.hj = [HB + jnp.minimum(j, n0 + 1) for j in range(nterms)]
                    self.ui = [jnp.maximum(n0 + 1 - j + UB, 0) for j in range(nterms + 1)]
                self.zi = [a + Z[3] if zdyn else a for a in range(2)]
                self.gi = GS + Z[1]
                self.nterms = nterms
                self.total = (D // 8) * nterms
                self.idx = 0

            def load(self, slot, rows):
                return sp_scr[slot, rows, :B], sp_scr[slot, rows, B:]

            def term(self):
                r, j = (self.idx // self.nterms) * 8, self.idx % self.nterms
                self.idx += 1
                rows = pl.ds(r, 8)
                hr, hi = self.load(self.hj[j], rows)
                u = [self.load(self.ui[j + 1], rows), self.load(self.ui[0], rows) if j == 0 else self.prev]
                self.prev = u[0]
                if j == 0:
                    self.acc = [(ur * hr - ui * hi, ur * hi + ui * hr) for (ur, ui) in u]
                else:
                    self.acc = [((ar + ur * hr) - ui * hi, (ai + ur * hi) + ui * hr)
                                for (ar, ai), (ur, ui) in zip(self.acc, u)]
                if j == self.nterms - 1:
                    for a in range(2):
                        z_scr[self.zi[a], rows, :B] = self.acc[a][0]
                        z_scr[self.zi[a], rows, B:] = self.acc[a][1]

            def run(self, toks, frac):
                for t, tok in sorted(toks, key=lambda x: x[0]):
                    tgt = int(round(self.total * frac(t)))
                    if self.idx < tgt:
                        sp_scr[self.gi, 0:8, 0:B] = tok()
                    while self.idx < tgt:
                        self.term()

            def finish(self):
                while self.idx < self.total:
                    self.term()

        XOP = {1: (0, 0), 3: (0, 1), 2: (1, 0), 4: (1, 1), 0: (1, 2), 6: (1, 3), 5: (1, 4)}

        def pacer(buf, toks, win, n):
            sel = [tok for (t, tok) in sorted(toks or [], key=lambda x: x[0]) if win[0] <= t < win[1]] if toks else []

            def pace(i):
                if sel:
                    buf[3 + Z[1], 0:8, :] = sel[min(i * len(sel) // n, len(sel) - 1)]()
            return pace

        def norm_pass(bufs2, t, mean, rstd, lg, toks=None, win=None):
            buf = bufs2[t]
            obuf, nbuf = xo[id(bufs2)]
            pace = pacer(buf, toks, win, D // lg)
            src = [1 + Z[2], 1 + Z[3]]
            hg = lg // 2
            for i, r in enumerate(range(0, DH, hg)):
                pace(i)
                lo = (buf[src[i % 2], r:r + hg, :] - mean) * rstd
                hi = (buf[src[i % 2], DH + r:DH + r + hg, :] - mean) * rstd
                if t == 0:
                    nbuf[Z[4] if xdyn else 0, r:r + hg, :] = lo
                    nbuf[Z[4] if xdyn else 0, DH + r:DH + r + hg, :] = hi
                    ops = [lo, hi - lo]
                else:
                    b11 = nbuf[Z[6], r:r + hg, :]
                    b21 = nbuf[Z[6], DH + r:DH + r + hg, :]
                    ops = [lo - hi, hi, b11 + hi, b21 + hi, b11 + lo]
                for k, o in enumerate(ops):
                    if xb16:
                        obuf[t][k + (Z[4] if xdyn else 0), r:r + hg, :] = o.astype(bf16)
                    else:
                        obuf[t][k + Z[4], r // 2:(r + hg) // 2, :] = _pk(o.astype(bf16))

        def load_xop(bufs2, p):
            t, k = XOP[p]
            return _upk(xo[id(bufs2)][0][t].bitcast(u32)[k + (Z[5] if xdyn else 0)])

        def q_stats(c):
            res = []
            for t in range(2):
                sq = None
                for r in range(0, D, 16):
                    q = q_buf[c, r:r + 16, t * B:(t + 1) * B].astype(f32)
                    sq = _Stats(q[0:1]) if sq is None else sq
                    sq.add(q)
                res.append(sq.done())
            return res

        def conv_inv(c, qs, lg, zs=None, t0=0, defer=False):
            inv = inv_ref[...]
            means = []
            toks = []
            par, cq, d0, d1 = c % 2, c + Z[6], Z[4], 1 + Z[4]
            for t in range(2):
                cols = slice(t * B, (t + 1) * B)
                mq, rq = qs[t]
                yc = _dot((z_scr[t + Z[3] if zdyn else t] if zs is None else zs[t]).astype(bf16), inv)
                s1 = _Stats(mq)
                for r in range(0, D, 16):
                    y = yc[r:r + 16] + kd_scr[par, r:r + 16, cols]
                    q = q_buf[cq, r:r + 16, cols].astype(f32)
                    x1 = q + ((q - mq) * rq) * y
                    la[t][d0, r:r + 16, :] = y
                    la[t][d1, r:r + 16, :] = x1
                    s1.add(x1)
                m1, r1 = s1.done()
                if defer:
                    means.append((m1, r1))
                    if t == 0:
                        toks += [(t0 + g * 16, rows_tok(yc, g)) for g in range(D // 16)]
                else:
                    norm_pass(la, t, m1, r1, lg)
                    means.append(m1)
            return (means, toks) if defer else means

        def first_conv(kv):
            never = Z[0] > 0
            qs = q_stats(0)
            fwd = fwd_ref[...]
            hs = []
            for a in range(2):
                hb = h_buf[0, :, a * B:(a + 1) * B]
                tok = _upk(_pk(jnp.broadcast_to(qs[a][1], (8, B))))
                hh = _dot(jnp.concatenate([hb[:D - 16], jnp.where(never, tok, hb[D - 16:])], axis=0), fwd)
                sp_scr[HB + a] = hh
                hs.append((hh[:, :B], hh[:, B:]))
            u0, u1 = _dot(kv[0], fwd), _dot(kv[1], fwd)
            sgn = alt_sign()
            a0 = (u0[:, :B], u0[:, B:])
            a1 = (u1[:, :B] - sgn * u0[:, B:], u1[:, B:] + sgn * u0[:, :B])
            sp_scr[UB] = u0
            sp_scr[UB + 1, :, :B] = a1[0]
            sp_scr[UB + 1, :, B:] = a1[1]
            uprev_scr[...] = u1

            def cmul(x, y):
                return x[0] * y[0] - x[1] * y[1], x[0] * y[1] + x[1] * y[0]
            z0 = cmul(a0, hs[0])
            p, q = cmul(a1, hs[0]), cmul(a0, hs[1])
            z1 = (p[0] + q[0], p[1] + q[1])
            return conv_inv(0, qs, D, zs=[jnp.concatenate(z, axis=1) for z in (z0, z1)])

        def mid_x3(t, st2, toks=None, win=None, LG=LG):
            pace = pacer(lx[t], toks, win, D // LG)
            ysrc, yslot = la[t], Z[7]
            m2, r2 = st2.done()
            st = _Stats(m2)
            d1 = 1 + Z[4]
            for i, r in enumerate(range(0, D, LG)):
                pace(i)
                x2 = lx[t][Z[2], r:r + LG, :]
                x3 = x2 + ((x2 - m2) * r2) * ysrc[yslot, r:r + LG, :]
                lb[t][d1, r:r + LG, :] = x3
                st.add(x3)
            return st

        def save_stats(t, st):
            st_scr[3 * t] = st.s1
            st_scr[3 * t + 1] = st.s2
            st_scr[3 * t + 2] = jnp.broadcast_to(st.c, (8, B))

        def load_stats(t):
            return _Stats(st_scr[3 * t + 2][0:1], st_scr[3 * t], st_scr[3 * t + 1])

        def rows_tok(x, g):
            return lambda: x[g * 16 + 8:g * 16 + 16]

        def a1_rows(p, r0, r1, gates=None, never=None, dyn=True):
            w = a1_scr.at[p + Z[7] if dyn else p]
            parts = []
            start = r0 // 16
            ng = r1 // 16
            for g in sorted(gates or {}) + [ng]:
                if g > start:
                    parts.append(w[start * 8:g * 8, :])
                if g < ng:
                    x = w[g * 8:(g + 1) * 8, :]
                    parts.append(jnp.concatenate([jnp.where(never, gates[g], x[:, :128]), x[:, 128:]], axis=1))
                start = g + 1
            return jnp.concatenate(parts, axis=0) if len(parts) > 1 else parts[0]

        HOP = {0: (0, 2), 1: (0, 1), 4: (0, 0), 2: (1, 0), 5: (1, 1), 3: (1, 2), 6: (1, 3)}

        def put_hop(l, p, r0, r1, v):
            cls, k = HOP[p]
            hid[l][cls][k, r0:r1, :] = v.astype(bf16)

        def get_hop(l, p, r0, r1):
            cls, k = HOP[p]
            return _upk(hid[l][cls].bitcast(u32)[k, r0 // 2:r1 // 2, :])

        def mm1(xb, l, t0=0, lhs=None, r0=0, r1=FH, gates=None, never=None, hooks=None, split0=1):
            n = r1 - r0
            gates = gates or {}
            hooks = hooks or {}

            def prod(p, rnd, a=r0, b=r1):
                gt = {g: tk for g, tk in gates.get(rnd, {}).items() if a // 16 <= g < b // 16} if p in (1, 2, 0) else {}
                w = a1_rows(p, a, b, gt, never, dyn1[l]) if lhs is None else lhs[p][(a - r0) // 2:(b - r0) // 2]
                return _dot(_upk(w), load_xop(xb, p))

            def toks(x, rnd, scale=1):
                return [(t0 + rnd * n + g * 16 // scale, rows_tok(x, g)) for g in range(n // 16)]
            if not (stage and lhs is None):
                m2, m4 = prod(1, 0), prod(3, 0)
                h21 = _silu(m2 + m4)
                put_hop(l, 4, r0, r1, h21)
                out = toks(h21, 0)
                hooks.get(0, lambda tk: None)(out)
                m3, m5 = prod(2, 1), prod(4, 1)
                h12 = _silu(m3 + m5)
                put_hop(l, 1, r0, r1, h12)
                put_hop(l, 0, r0, r1, h12 + h21)
                p11, p22 = m4 - m5, m3 - m2
                out += toks(h12, 1)
                hooks.get(1, lambda tk: None)(out)
                m1, m7 = prod(0, 2), prod(6, 2)
                h11 = _silu((p11 + m1) + m7)
                p22 = p22 + m1
                put_hop(l, 2, r0, r1, h11 - h21)
                put_hop(l, 5, r0, r1, h12 + h11)
                out += toks(h11, 2)
                mid = r0 + n // 2
                h22a = _silu(p22[:n // 2] + prod(5, 3, r0, mid))
                h22b = _silu(p22[n // 2:] + prod(5, 3, mid, r1))
                h22 = jnp.concatenate([h22a, h22b], axis=0)
                put_hop(l, 3, r0, r1, h22 - h12)
                put_hop(l, 6, r0, r1, h22 + h21)
                out += [(t0 + 3 * n + g * 16, rows_tok(h22a, g)) for g in range(n // 32)]
                return out

            wr = [k + Z[2] for k in range(5)]
            rd = [k + Z[3] for k in range(4)]
            m2, m4 = prod(1, 0), prod(3, 0)
            h21 = _silu(m2 + m4)
            put_hop(l, 4, 0, n, h21)
            pp[wr[0]] = m4
            pp[wr[1]] = m2
            pp[wr[2]] = h21
            out = toks(h21, 0)
            hooks.get(0, lambda tk: None)(out)
            m3, m5 = prod(2, 1), prod(4, 1)
            h12 = _silu(m3 + m5)
            put_hop(l, 1, 0, n, h12)
            pp[wr[4], 0:8, :] = m3[0:8]
            for a in range(0, n, G):
                b = a + G
                x4, x2, x21 = pp[rd[0], a:b, :], pp[rd[1], a:b, :], pp[rd[2], a:b, :]
                put_hop(l, 0, a, b, h12[a:b] + x21)
                pp[wr[0], a:b, :] = x4 - m5[a:b]
                pp[wr[1], a:b, :] = m3[a:b] - x2
                pp[wr[3], a:b, :] = h12[a:b]
            out += toks(h12, 1)
            m1, m7 = prod(0, 2), prod(6, 2)
            pp[wr[4], 0:8, :] = m1[0:8]
            hs = []
            for a in range(0, n, G):
                b = a + G
                p11, p22 = pp[rd[0], a:b, :], pp[rd[1], a:b, :]
                x21, x12 = pp[rd[2], a:b, :], pp[rd[3], a:b, :]
                h11 = _silu((p11 + m1[a:b]) + m7[a:b])
                put_hop(l, 2, a, b, h11 - x21)
                put_hop(l, 5, a, b, x12 + h11)
                pp[wr[1], a:b, :] = p22 + m1[a:b]
                hs.append(h11)
            out += toks(jnp.concatenate(hs, axis=0), 2)
            m6 = [prod(5, 3, 0, n // 2), prod(5, 3, n // 2, n)]
            hs = []
            for a0 in range(0, n // 2, G // 2):
                pp[wr[4], 0:8, :] = m6[0][max(a0 - 8, 0):max(a0 - 8, 0) + 8]
                for hf in range(2):
                    a = hf * (n // 2) + a0
                    b = a + G // 2
                    h22 = _silu(pp[rd[1], a:b, :] + m6[hf][a0:a0 + G // 2])
                    put_hop(l, 3, a, b, h22 - pp[rd[3], a:b, :])
                    put_hop(l, 6, a, b, h22 + pp[rd[2], a:b, :])
                    if hf == 0:
                        hs.append(h22)
            h22a = jnp.concatenate(hs, axis=0)
            out += [(t0 + 3 * n + g * 16, rows_tok(h22a, g)) for g in range(n // 32)]
            return out

        def mm2(l, t0, res, tile_done, lhs=None, pop_from=99):
            toks = []
            M = {}
            ch = _chunks2()
            never = Z[0] > 0
            prev_round, cur_round = [], []
            for i, (p, ka, kb, rnd) in enumerate(ch):
                first_in_round = i == 0 or ch[i - 1][3] != rnd
                if first_in_round:
                    prev_round, cur_round = cur_round, []
                w = a2_scr[p + Z[7] if (dyn2[l] and MODE['mac']) else p, :, ka * 128:kb * 128] if lhs is None else lhs[p][:, ka * 128:kb * 128]
                if first_in_round and rnd >= pop_from:
                    parts = []
                    start = 0
                    for g, gp in ((0, 5), (4, 9), (8, 13)):
                        tk = None
                        for x in prev_round:
                            y = _pk(rows_tok(x, gp)())
                            tk = y if tk is None else tk | y
                        if g > start:
                            parts.append(w[start * 8:g * 8])
                        x = w[g * 8:(g + 1) * 8]
                        x0 = jnp.where(never, tk, x[:, :128])
                        parts.append(jnp.concatenate([x0, x[:, 128:]], axis=1) if x.shape[1] > 128 else x0)
                        start = g + 1
                    parts.append(w[start * 8:])
                    w = jnp.concatenate(parts, axis=0)
                w = _upk(w)
                hb = get_hop(l, p, ka * 128, kb * 128)
                if i == len(ch) - 1:
                    r = jnp.concatenate([_dot(w[a:b], hb) for a, b in ((0, 64), (64, 128), (128, 176), (176, DH))],
                                        axis=0)
                else:
                    r = _dot(w, hb)
                if p not in M:
                    if p == 5:
                        r = (((res(0, 1) + M[0]) - M[1]) + M[2]) + r
                    elif p == 6:
                        r = (((res(1, 0) + M[0]) - M[4]) + M[3]) + r
                    M[p] = r
                else:
                    M[p] = M[p] + r
                cur_round.append(M[p])
                if first_in_round:
                    toks += [(t0 + rnd * DH + g * 16, rows_tok(M[p], g)) for g in range(DH // 16)]
                if p == 5 and kb == 7:
                    tile_done(0, (res(0, 0) + M[4]) + M[2], M[5], (0, 1))
            tile_done(1, M[6], (res(1, 1) + M[1]) + M[3], (1, 0))
            return toks

        def ffn1_out(means, t0, lhs=None, fast=False):
            def fin(t, lo, hi, order):
                st = _Stats(means[t])
                for h in order:
                    x2 = (lo, hi)[h]
                    lx[t][Z[4], h * DH:(h + 1) * DH, :] = x2
                    st.add(x2, (0, 64, 128, 176, DH) if (t == 1 and h == 0 and NCH > 1) else None)
                sts[t] = st
            sts = {}
            toks = mm2(0, t0, lambda t, h: la[t][1 + Z[6], h * DH:(h + 1) * DH, :], fin, lhs, popg)
            if fast:
                st3 = mid_x3(0, sts[0], toks, (t0 + FX[0], t0 + FX[1]), LG)
                norm_pass(lb, 0, *st3.done(), LG, toks, (t0 + FX[2], t0 + FX[3]))
            else:
                save_stats(0, mid_x3(0, sts[0], toks, (t0 + PX0[0], t0 + PX0[1])))
            save_stats(1, sts[1])
            return toks

        def ffn2_out(m, t0, last):
            def fin(t, lo, hi, order):
                for h in order:
                    o_buf[2 * m + t, h * DH:(h + 1) * DH] = (lo, hi)[h].astype(bf16)
                    if last and t == 1:
                        out_copy(m, t, h * DH, (h + 1) * DH).start()
                if not (last and t == 1):
                    out_copy(m, t, 0, D).start()
            return mm2(1, t0, lambda t, h: lb[t][1 + Z[6], h * DH:(h + 1) * DH, :], fin, None, popg4)

        def w1_operands(src, c0):
            parts = [[] for _ in range(7)]
            for c in range(0, src.shape[2], 128):
                blk = [src[i, k * DH:(k + 1) * DH, c:c + 128].T for i in range(2) for k in range(2)]
                for p, wp in enumerate(_strassen_lhs(*blk)):
                    a1_scr[p, (c0 + c) // 2:(c0 + c + 128) // 2, :] = wp
                    parts[p].append(wp)
            return [jnp.concatenate(x, axis=0) for x in parts]

        def prologue():
            order = [cp_sk, cp_dd, blk_copy(1, 0), blk_copy(2, 0), cp_fwd, blk_copy(3, 0), blk_copy(0, 0)] \
                + cp_w1a + [blk_copy(3, 1), blk_copy(1, 1), blk_copy(2, 1)] + cp_w1b + [cp_w2]
            for c in range(1, NSTEP):
                order.append(blk_copy(0, c))
                if c + 1 < NSTEP:
                    order += [blk_copy(w, c + 1) for w in (1, 2, 3)]
            for cp in order:
                cp.start()
            for i in range(NFLAG):
                flag_scr[i] = 0
            sp_scr[0] = jnp.zeros((D, 2 * B), f32)

            wait_all("w_small", [cp_sk, cp_dd])
            sk = sk_ref[...].astype(f32)
            dd = dd_ref[...].astype(f32).reshape(1, D)
            pt = jnp.concatenate([sk, dd, jnp.zeros((3, D), f32)], axis=0).T
            for j in range(5):
                taps_scr[j] = jnp.broadcast_to(pt[:, j:j + 1], (D, B))

            wait_all("w_kv0", [blk_copy(1, 0), blk_copy(2, 0)])
            kv0 = conv_kv(0)[0]

            wait_all("w_blk0", [cp_fwd, blk_copy(3, 0), blk_copy(0, 0)])
            inv_ref[...] = (fwd_ref[...].astype(f32).T * (1.0 / B)).astype(bf16)
            means0 = first_conv(kv0)

            wait_all("w_w1a", cp_w1a)
            mm1(la, 0, lhs=w1_operands(w1a_ref, 0), r1=WA)

            wait_all("w_w1b", [blk_copy(3, 1), blk_copy(1, 1), blk_copy(2, 1)] + cp_w1b)
            conv_fwd_h(1)
            kv1 = conv_kv(1)[0]
            toks0 = mm1(la, 0, lhs=w1_operands(w1b_ref, WA), r0=WA, hooks={1: lambda tk: conv_fwd_u(1, kv1)})
            nb = FH - WA
            mac1 = Mac(1, 4)
            mac1.run([x for x in toks0 if x[0] >= 2 * nb], lambda t: mfrac * (t - 2 * nb) / (1.5 * nb))

            wait_all("w_w2", [cp_w2])
            lhs2 = _strassen_lhs(w2_ref[:DH, :FH], w2_ref[:DH, FH:], w2_ref[DH:, :FH], w2_ref[DH:, FH:])
            for p in range(7):
                a2_scr[p] = lhs2[p]
            toks0 = ffn1_out(means0, 0, lhs2)
            mac1.run(toks0, lambda t: min(1.0, mfrac + (1 - mfrac) * t / 1800))
            mac1.finish()

            wait_all("w_blk2", [blk_copy(0, 1)] + [blk_copy(w, 2) for w in (1, 2, 3)])

        def body(m, nxt, fwd):
            load_flags()
            MODE['mac'] = fwd or d2tail
            never = Z[0] > 0
            t3 = (TC if nxt else 0) + (TC if fwd else 0)
            t4 = t3 + T1 + (TC if fwd else 0)
            gates = {0: {}, 1: {}, 2: {}}

            def deadline(tok, t):
                d, g = gates[(t - t3) // FH], ((t - t3) % FH) // 16
                d[g] = tok if g not in d else d[g] | tok

            def frac(t):
                return sum(w * max(0, min(b, t) - a) for a, b, w in REL) / sum(w * (b - a) for a, b, w in REL)

            if nxt:
                qs = q_stats(m + 1)
            if fwd:
                th = conv_fwd_h(m + 2, [(Q_GATE[t] // 16, _pk(jnp.broadcast_to(qs[t][1], (8, B)))) for t in range(2)],
                                never)
                norm_pass(lb, 0, *load_stats(0).done(), LG, th, PN0)
                st3 = mid_x3(1, load_stats(1), th, PX1)
                mr, ti = conv_inv(m + 1, qs, LG, t0=TC, defer=True)
                kv, toks = conv_kv(m + 2)
                for i, tok in enumerate(toks):
                    deadline(tok, int(KV_WIN[0] + (KV_WIN[1] - KV_WIN[0]) * (i + 1) / len(toks)))
                toks = mm1(lb, 1, t3, gates=gates, never=never,
                           hooks={0: lambda tk: norm_pass(lb, 1, *st3.done(), LG, ti + tk, PN1)})
            else:
                res = {}
                if nxt:
                    norm_pass(lb, 0, *load_stats(0).done(), D)
                    for t in range(2):
                        gates[0][TQ[t] // 16] = _pk(jnp.broadcast_to(qs[t][1], (8, B)))

                def hook(tk):
                    st3 = mid_x3(1, load_stats(1), tk, TX[0:2])
                    ti = []
                    if nxt:
                        res["mr"], ti = conv_inv(m + 1, qs, LG, t0=FH, defer=True)
                    norm_pass(lb, 1, *st3.done(), LG, tk + ti, TX[2:4] if nxt else TX[4:6])
                toks = mm1(lb, 1, 0, gates=gates, never=never, hooks={0: hook})
                toks = [(t + (TC if (nxt and t >= FH) else 0), tok) for t, tok in toks]
                mr = res.get("mr")
            if nxt:
                means = [x[0] for x in mr]
            if fwd:
                toks += conv_fwd_u(m + 2, kv, t3 + T1)
                mac = Mac(m + 2, NB)
            toks4 = ffn2_out(m, t4, not nxt)
            if nxt:
                half = (PNA[0] + PNA[1]) // 2
                sh2 = 0 if fwd else -2 * TC
                norm_pass(la, 0, *mr[0], LG, toks + toks4, (PNA[0] + sh2, half + sh2))
                norm_pass(la, 1, *mr[1], LG, toks + toks4, (half + sh2, PNA[1] + sh2))
            toks = toks4
            if fwd:
                mac.run(toks, frac)
            if nxt:
                toks = mm1(la, 0, t4 + T2)
                if fwd:
                    mac.run(toks, frac)
                toks = ffn1_out(means, t4 + T2 + T1, fast=not fwd)
                if fwd:
                    mac.run(toks, frac)
                    mac.finish()

        scoped("prologue", prologue)

        def step(m, carry):
            @pl.when(m == 1)
            def _():
                for w in range(4):
                    for c in range(2 if w == 0 else 3, NSTEP):
                        blk_copy(w, c).wait()

            scoped("main", lambda: body(m, True, True))
            return carry

        jax.lax.fori_loop(0, NSTEP - 2, step, 0)

        def tail():
            body(NSTEP - 2, True, False)
            body(NSTEP - 1, False, False)
        scoped("last", tail)
        for c in range(NSTEP):
            for t in range(2):
                for r0, r1 in out_rows((c, t) == (NSTEP - 1, 1)):
                    out_copy(c, t, r0, r1).wait()

    @jax.jit
    def run(A_q, A_k, A_v, A_shift_k, A_ssm_k, A_ssm_D, B_x, B_w1, B_w2):
        qT = jnp.swapaxes(A_q, 1, 2).reshape(D, S)
        kT = jnp.swapaxes(A_k, 1, 2).reshape(D, S)
        vT = jnp.swapaxes(A_v, 1, 2).reshape(D, S)
        anyspec = pl.BlockSpec(memory_space=pl.ANY)
        blocks = pltpu.VMEM((NSTEP, D, TM), bf16)
        hbuf = lambda n: pltpu.VMEM((n, FH, B), bf16)
        lnbuf = pltpu.VMEM((4, D, B), f32)
        xbuf = (lambda n: pltpu.VMEM((n, DH, B), bf16)) if xb16 else (lambda n: pltpu.VMEM((n, DH // 2, B), u32))
        out = pl.pallas_call(
            _kernel,
            in_specs=[anyspec] * 9,
            out_specs=anyspec,
            out_shape=jax.ShapeDtypeStruct((D, S), bf16),
            scratch_shapes=[
                blocks, blocks, blocks, blocks,
                pltpu.VMEM((4, D), bf16), pltpu.VMEM((D,), bf16),
                pltpu.VMEM((2, D, WA), bf16), pltpu.VMEM((2, D, FH - WA), bf16),
                pltpu.VMEM((D, F), bf16),
                pltpu.VMEM((B, 2 * B), bf16), pltpu.VMEM((2 * B, B), bf16),
                pltpu.VMEM((2 * NSTEP, D, B), bf16),
                pltpu.VMEM((NSLOT, D, 2 * B), f32),
                pltpu.VMEM((2, D, TM), f32),
                pltpu.VMEM((D, 2 * B), f32),
                pltpu.VMEM((5, D, B), f32),
                pltpu.VMEM((7, FH // 2, DH), u32),
                pltpu.VMEM((7, DH // 2, FH), u32),
                hbuf(3), hbuf(4), hbuf(3), hbuf(4),
                pltpu.VMEM((5, FH, B), f32),
                xbuf(2), xbuf(5), xbuf(2), xbuf(5), pltpu.VMEM((1, D, B), f32), pltpu.VMEM((1, D, B), f32),
                lnbuf, lnbuf, lnbuf, lnbuf, lnbuf, lnbuf,
                pltpu.VMEM((6, 8, B), f32),
                pltpu.VMEM((2, D, 2 * B), f32),
                pltpu.SMEM((NFLAG,), jnp.int32),
                pltpu.SemaphoreType.DMA((8,)),
                pltpu.SemaphoreType.DMA((1,)),
            ],
            compiler_params=pltpu.CompilerParams(vmem_limit_bytes=100 * 1024 * 1024),
            interpret=interp,
        )(qT, kT, vT, A_ssm_k, A_shift_k.T, A_ssm_D, B_w1, B_w2.T, _dft_table())
        return jnp.swapaxes(out.reshape(1, D, S), 1, 2)
    return run


_impl = make()


@jax.jit
def pallas_interleave_layers__ssm_conv_h3__dense_activation_silu__prompt_kernel(
    A_q: jax.Array,
    A_k: jax.Array,
    A_v: jax.Array,
    A_shift_k: jax.Array,
    A_ssm_k: jax.Array,
    A_ssm_D: jax.Array,
    B_x: jax.Array,
    B_w1: jax.Array,
    B_w2: jax.Array,
):
    return _impl(A_q, A_k, A_v, A_shift_k, A_ssm_k, A_ssm_D, B_x, B_w1, B_w2)
```
